```python
import jax
import jax.numpy as jnp

def _softmax(x, axis=-1):
    return jax.nn.softmax(x, axis=axis)

def _gelu(x):
    return jax.nn.gelu(x, approximate=True)

def _silu(x):
    return jax.nn.silu(x)

def _sigmoid(x):
    return jax.nn.sigmoid(x)

def _layernorm(x, axis=-1, eps=1e-05):
    m = jnp.mean(x, axis=axis, keepdims=True)
    v = jnp.var(x, axis=axis, keepdims=True)
    return (x - m) / jnp.sqrt(v + eps)

def _scatter_add(tgt, idx, src, axis=0):
    return tgt.at[idx].add(src)

def _segment_sum(src, seg, n):
    return jax.ops.segment_sum(src, seg, n)

class _Rng:

    def __init__(self, key):
        self._k = key

    def _next(self):
        self._k, sub = jax.random.split(self._k)
        return sub

    def normal(self, shape):
        return jax.random.normal(self._next(), shape, dtype=jnp.bfloat16)

    def randint(self, lo, hi, shape):
        return jax.random.randint(self._next(), shape, lo, hi, dtype=jnp.int32)

    def uniform(self, shape, lo=0.0, hi=1.0):
        return jax.random.uniform(self._next(), shape, jnp.bfloat16, lo, hi)

    def permutation(self, n):
        return jax.random.permutation(self._next(), n)
kernel_name = 'standalone__conformer_family_conformer__speech'

def setup_inputs():
    _rng = _Rng(jax.random.key(int.from_bytes(__import__("os").urandom(4), "little")))
    _w = lambda a: (lambda t: t.astype(jnp.bfloat16) if jnp.issubdtype(t.dtype, jnp.floating) else t)(jnp.asarray(a))
    B, T, D, K = (2, 4000, 512, 15)
    F = 4 * D
    s = D ** (-0.5)
    sf = F ** (-0.5)
    return {'x': _w((lambda *s: _rng.normal(s) * 0.05)(B, T, D)), 'w_ff1_a': _w((lambda *s: _rng.normal(s) * 0.05)(D, F) * s), 'w_ff1_b': _w((lambda *s: _rng.normal(s) * 0.05)(F, D) * sf), 'w_q': _w((lambda *s: _rng.normal(s) * 0.05)(D, D) * s), 'w_k': _w((lambda *s: _rng.normal(s) * 0.05)(D, D) * s), 'w_v': _w((lambda *s: _rng.normal(s) * 0.05)(D, D) * s), 'w_o': _w((lambda *s: _rng.normal(s) * 0.05)(D, D) * s), 'w_pw1': _w((lambda *s: _rng.normal(s) * 0.05)(D, 2 * D) * s), 'dw': _w((lambda *s: _rng.normal(s) * 0.05)(K, D) * K ** (-0.5)), 'w_pw2': _w((lambda *s: _rng.normal(s) * 0.05)(D, D) * s), 'w_ff2_a': _w((lambda *s: _rng.normal(s) * 0.05)(D, F) * s), 'w_ff2_b': _w((lambda *s: _rng.normal(s) * 0.05)(F, D) * sf)}

def reference(x, w_ff1_a, w_ff1_b, w_q, w_k, w_v, w_o, w_pw1, dw, w_pw2, w_ff2_a, w_ff2_b):
    B, T, D = x.shape
    K = dw.shape[0]
    scale = D ** (-0.5)
    h = _layernorm(x, axis=-1)
    h = _silu(h @ w_ff1_a) @ w_ff1_b
    x1 = x + 0.5 * h
    h = _layernorm(x1, axis=-1)
    q = h @ w_q
    k = h @ w_k
    v = h @ w_v
    scores = jnp.einsum('btd,bsd->bts', q, k) * scale
    p = _softmax(scores, axis=-1)
    attn = jnp.einsum('bts,bsd->btd', p, v) @ w_o
    x2 = x1 + attn
    h = _layernorm(x2, axis=-1)
    h = h @ w_pw1
    a = h[..., :D].copy()
    b = h[..., D:].copy()
    h = a * _sigmoid(b)
    pad = K // 2
    hp = jnp.pad(h, ((0, 0), (pad, K - 1 - pad), (0, 0)))
    dc = jnp.zeros_like(h)
    for i in range(K):
        dc = dc + hp[:, i:i + T, :] * dw[i][None, None, :]
    flat = dc.reshape(-1, D)
    mu = flat.mean(0)
    var = ((flat - mu) ** 2).mean(0)
    dc = (dc - mu[None, None, :]) / jnp.sqrt(var[None, None, :] + 1e-05)
    h = _silu(dc) @ w_pw2
    x3 = x2 + h
    h = _layernorm(x3, axis=-1)
    h = _silu(h @ w_ff2_a) @ w_ff2_b
    x4 = x3 + 0.5 * h
    return _layernorm(x4, axis=-1)
```

```python
import functools
import jax
import jax.numpy as jnp
import numpy as np
import jax.experimental.pallas as pl
import jax.experimental.pallas.tpu as pltpu

B, T, D, F, KW = 2, 4000, 512, 2048, 15
TP = 4096
BF = jnp.bfloat16
F32 = jnp.float32
EPS = 1e-5
LOG2E = 1.4426950408889634

TM1 = 400
TQ = 400
TM3 = 400
KC = 1024
HALO = 8


def _ln(x):
  m = jnp.mean(x, axis=-1, keepdims=True)
  xc = x - m
  v = jnp.mean(xc * xc, axis=-1, keepdims=True)
  return xc * jax.lax.rsqrt(v + EPS)


def _silu(z):
  hz = 0.5 * z
  return hz + hz * jnp.tanh(hz)


def _dot(a, b):
  return jnp.dot(a, b, preferred_element_type=F32)


def _dot_nt(a, b):
  return jax.lax.dot_general(a, b, (((1,), (1,)), ((), ())), preferred_element_type=F32)


def kernel(x_ref, wa1, wb1, wq, wk, wv, wo, wp1, dw_ref, wp2, wa2, wb2, out_ref,
           mqk, mvo, x1_ref, h1_ref, g_ref, dc_ref, st_ref):
  scale = D ** -0.5 * LOG2E
  mqk[...] = (_dot_nt(wq[...], wk[...]) * scale).astype(BF)
  mvo[...] = _dot(wv[...], wo[...]).astype(BF)

  for b in range(B):
    h1_ref[b, T:TP, :] = jnp.zeros((TP - T, D), BF)
    g_ref[b, 0:HALO, :] = jnp.zeros((HALO, D), F32)
    g_ref[b, HALO + T:HALO + T + 8, :] = jnp.zeros((8, D), F32)

  def p1(i, _):
    b = i // (T // TM1)
    r = pl.multiple_of((i % (T // TM1)) * TM1, TM1)
    x = x_ref[b, pl.ds(r, TM1), :].astype(F32)
    h = _ln(x).astype(BF)
    z = _dot(h, wa1[...])
    s = _silu(z).astype(BF)
    y = _dot(s, wb1[...])
    x1 = x + 0.5 * y
    x1_ref[b, pl.ds(r, TM1), :] = x1
    h1_ref[b, pl.ds(r, TM1), :] = _ln(x1).astype(BF)
    return _
  jax.lax.fori_loop(0, B * T // TM1, p1, 0)

  def p2(i, _):
    b = i // (T // TQ)
    r = pl.multiple_of((i % (T // TQ)) * TQ, TQ)
    hq = h1_ref[b, pl.ds(r, TQ), :]
    q = _dot(hq, mqk[...]).astype(BF)
    m = jnp.full((TQ, 1), -1e30, F32)
    l = jnp.zeros((TQ, 1), F32)
    acc = jnp.zeros((TQ, D), F32)
    for c in range(TP // KC):
      kk = h1_ref[b, c * KC:(c + 1) * KC, :]
      s = _dot_nt(q, kk)
      if (c + 1) * KC > T:
        col = jax.lax.broadcasted_iota(jnp.int32, (TQ, KC), 1) + c * KC
        s = jnp.where(col < T, s, -1e30)
      mn = jnp.maximum(m, jnp.max(s, axis=-1, keepdims=True))
      p = jnp.exp2(s - mn)
      al = jnp.exp2(m - mn)
      l = l * al + jnp.sum(p, axis=-1, keepdims=True)
      acc = acc * al + _dot(p.astype(BF), kk)
      m = mn
    o = (acc * (1.0 / l)).astype(BF)
    x2 = x1_ref[b, pl.ds(r, TQ), :] + _dot(o, mvo[...])
    x1_ref[b, pl.ds(r, TQ), :] = x2
    h = _ln(x2).astype(BF)
    ab = _dot(h, wp1[...])
    a = ab[:, :D]
    bb = ab[:, D:]
    gl = a * (0.5 + 0.5 * jnp.tanh(0.5 * bb))
    g_ref[b, pl.ds(r + HALO, TQ), :] = gl
    return _
  jax.lax.fori_loop(0, B * T // TQ, p2, 0)

  TC = 400
  dw = dw_ref[...].astype(F32)

  st_ref[...] = jnp.zeros((16, D), F32)
  def pc(i, carry):
    b = i // (T // TC)
    r = pl.multiple_of((i % (T // TC)) * TC, TC)
    acc = jnp.zeros((TC, D), F32)
    w = g_ref[b, pl.ds(r, TC + 16), :]
    for k in range(KW):
      o = HALO - KW // 2 + k
      acc = acc + w[o:o + TC, :] * dw[k:k + 1, :]
    dc_ref[b, pl.ds(r, TC), :] = acc
    st_ref[0:8, :] += jnp.sum(acc.reshape(TC // 8, 8, D), axis=0)
    return carry
  jax.lax.fori_loop(0, B * T // TC, pc, 0)
  mu = jnp.sum(st_ref[0:8, :], axis=0, keepdims=True) * (1.0 / (B * T))

  def pv(i, carry):
    b = i // (T // TC)
    r = pl.multiple_of((i % (T // TC)) * TC, TC)
    d = dc_ref[b, pl.ds(r, TC), :] - mu
    st_ref[8:16, :] += jnp.sum((d * d).reshape(TC // 8, 8, D), axis=0)
    return carry
  jax.lax.fori_loop(0, B * T // TC, pv, 0)
  s2 = jnp.sum(st_ref[8:16, :], axis=0, keepdims=True)
  rs = jax.lax.rsqrt(s2 * (1.0 / (B * T)) + EPS)

  def p3(i, _):
    b = i // (T // TM3)
    r = pl.multiple_of((i % (T // TM3)) * TM3, TM3)
    dcn = (dc_ref[b, pl.ds(r, TM3), :] - mu) * rs
    hh = _silu(dcn).astype(BF)
    x3 = x1_ref[b, pl.ds(r, TM3), :] + _dot(hh, wp2[...])
    h = _ln(x3).astype(BF)
    z = _dot(h, wa2[...])
    s = _silu(z).astype(BF)
    y = _dot(s, wb2[...])
    x4 = x3 + 0.5 * y
    out_ref[b, pl.ds(r, TM3), :] = _ln(x4).astype(out_ref.dtype)
    return _
  jax.lax.fori_loop(0, B * T // TM3, p3, 0)


@jax.jit
def pallas_standalone__conformer_family_conformer__speech_kernel(
    x, w_ff1_a, w_ff1_b, w_q, w_k, w_v, w_o, w_pw1, dw, w_pw2, w_ff2_a, w_ff2_b):
  vm = pl.BlockSpec(memory_space=pltpu.VMEM)
  return pl.pallas_call(
      kernel,
      out_shape=jax.ShapeDtypeStruct(x.shape, x.dtype),
      in_specs=[vm] * 12,
      out_specs=vm,
      scratch_shapes=[
          pltpu.VMEM((D, D), BF), pltpu.VMEM((D, D), BF),
          pltpu.VMEM((B, T, D), F32),
          pltpu.VMEM((B, TP, D), BF),
          pltpu.VMEM((B, T + 16, D), F32),
          pltpu.VMEM((B, T, D), F32),
          pltpu.VMEM((16, D), F32),
      ],
      compiler_params=pltpu.CompilerParams(vmem_limit_bytes=120 * 1024 * 1024),
  )(x, w_ff1_a, w_ff1_b, w_q, w_k, w_v, w_o, w_pw1, dw, w_pw2, w_ff2_a, w_ff2_b)
```

```python
import jax
import jax.numpy as jnp
import jax.experimental.pallas as pl
import jax.experimental.pallas.tpu as pltpu

BF = jnp.bfloat16
F32 = jnp.float32
U32 = jnp.uint32

NB, T, D, FH, KW = 2, 4000, 512, 2048, 15
N = NB * T
TM = 800
H = TM // 2
NT = N // TM
TPB = T // TM
EPS = 1e-5
QSCALE = D ** -0.5 * 1.4426950408889634
NEG = -1e30
CAP = 34

PVMAP = [0, 2, 6, 5, 3, 4, 1]
AORD = [4, 1, 0, 3, 2, 6, 5]
BORD = [2, 3, 0, 4, 6, 5, 1]
NEED = {2: [0], 3: [3], 0: [0, 3], 4: [0, 1], 6: [1, 3], 5: [2, 0], 1: [2, 3]}
CONTRIB = [((0, 1), (3, 1)), ((2, 1), (3, -1)), ((1, 1), (3, 1)), ((0, 1), (2, 1)),
           ((0, -1), (1, 1)), ((3, 1),), ((0, 1),)]


def dot(a, b):
  return jnp.dot(a, b, preferred_element_type=F32)


def dot_nt(a, b):
  return jax.lax.dot_general(a, b, (((1,), (1,)), ((), ())), preferred_element_type=F32)


def alpha_forms(a11, a12, a21, a22):
  return [lambda: a11 + a22, lambda: a21 + a22, lambda: a11, lambda: a22,
          lambda: a11 + a12, lambda: a21 - a11, lambda: a12 - a22]


def beta_forms(b11, b12, b21, b22):
  return [lambda: b11 + b22, lambda: b11, lambda: b12 - b22, lambda: b21 - b11,
          lambda: b22, lambda: b11 + b12, lambda: b21 + b22]


def phi_forms(q11, q12, q21, q22):
  return beta_forms(q11, q21, q12, q22)


def quads(ha, hb):
  return ha[:, :256], ha[:, 256:], hb[:, :256], hb[:, 256:]


class Gamma:
  def __init__(self, init=None, transposed=False):
    self.p = [None] * 4 if init is None else [(v, 1) for v in init]
    self.tr = transposed

  def add(self, j, m):
    for q, sg in CONTRIB[j]:
      if self.tr and q in (1, 2):
        q = 3 - q
      cur = self.p[q]
      if cur is None:
        self.p[q] = (m, sg)
      else:
        v, s = cur
        if s == 1:
          self.p[q] = (v + m if sg == 1 else v - m, 1)
        else:
          self.p[q] = (m - v, 1) if sg == 1 else (v + m, -1)

  def result(self):
    assert all(s == 1 for _, s in self.p)
    return [v for v, _ in self.p]


def rep(x, n, axis):
  return jnp.concatenate([x] * n, axis=axis) if n > 1 else x


def ld_bf(u):
  return pltpu.bitcast(u, BF)


def st_bf(x):
  return pltpu.bitcast(x.astype(BF), U32)


def ln_rows(x):
  m = jnp.mean(x, axis=-1, keepdims=True)
  xc = x - m
  v = jnp.mean(xc * xc, axis=-1, keepdims=True)
  return xc * jax.lax.rsqrt(v + EPS)


def half_silu(hz):
  return hz + hz * jnp.tanh(hz)


def row_vregs(x, c0=0):
  return [x[r:r + 8, c0:c0 + 128] for r in range(0, x.shape[0], 8)]


def tie(zm, u, deps, cast):
  if not deps:
    return u
  n = u.shape[0] // 8
  nk = u.shape[1] // 128
  slots = n * nk
  assign = {}
  for idx, d in enumerate(deps):
    assign[(idx * slots) // len(deps)] = d
  rows = []
  for rb in range(n):
    blk = u[rb * 8:(rb + 1) * 8]
    if any((rb * nk + k) in assign for k in range(nk)):
      parts = []
      for k in range(nk):
        pc = blk[:, k * 128:(k + 1) * 128]
        d = assign.get(rb * nk + k)
        if d is not None:
          pc = jnp.where(zm, pltpu.bitcast(d, U32) if cast else d, pc)
        parts.append(pc)
      blk = jnp.concatenate(parts, axis=1)
    rows.append(blk)
  return jnp.concatenate(rows, axis=0)


def interleave(a, b):
  out = []
  for i in range(max(len(a), len(b))):
    if i < len(a):
      out.append(a[i])
    if i < len(b):
      out.append(b[i])
  return out


def merge(s1, s2):
  out, n1, n2, i, j = [], len(s1), len(s2), 0, 0
  while i < n1 or j < n2:
    if j >= n2 or (i < n1 and i * n2 <= j * n1):
      out.append(s1[i]); i += 1
    else:
      out.append(s2[j]); j += 1
  return out


def kernel(x_h, wa1_h, wb1_h, wq_h, wk_h, wv_h, wo_h, wp1_h, dw_h, wp2_h, wa2_h, wb2_h, out_h,
           xo, ra1, rb1, ra2, rb2, rq, rk, rv, ro, rp1, rdw, rp2,
           WA, WB, MQK, MVO, WP1, WP2, DWB, x1, dc, G, gb, sS, qa, osc, lsc, st, bn, zs, sem):

  def xcopy(t):
    return pltpu.make_async_copy(x_h.at[pl.ds(t * TM, TM)], xo.at[pl.ds(t * TM, TM)], sem.at[t])

  def ocopy(t):
    return pltpu.make_async_copy(xo.at[pl.ds(t * TM, TM)], out_h.at[pl.ds(t * TM, TM)], sem.at[NT + 11 + t])

  wsrc = [wa1_h, wb1_h, wq_h, wk_h, wv_h, wo_h, wp1_h, dw_h, wp2_h, wa2_h, wb2_h]
  wdst = [ra1, rb1, rq, rk, rv, ro, rp1, rdw, rp2, ra2, rb2]
  I_A1, I_B1, I_Q, I_K, I_V, I_O, I_P1, I_DW, I_P2, I_A2, I_B2 = range(11)

  def wcopy(i):
    return pltpu.make_async_copy(wsrc[i], wdst[i], sem.at[NT + i])

  xcopy(0).start()
  wcopy(I_A1).start()
  wcopy(I_B1).start()
  xcopy(1).start()
  for i in (I_Q, I_K, I_V, I_O):
    wcopy(i).start()
  for t in range(2, NT):
    xcopy(t).start()
  for i in (I_P1, I_DW, I_P2, I_A2, I_B2):
    wcopy(i).start()

  def prep_weight(raw, dst, kh, nh, scale, cw=256):
    deps = []
    for c0 in range(0, nh, cw):
      for r0 in range(0, kh, 256):
        blk = [raw[r:r + 256, c:c + cw].astype(F32) * scale
               for r in (r0, kh + r0) for c in (c0, nh + c0)]
        for j, f in enumerate(beta_forms(*blk)):
          dst[j, r0 // 2:r0 // 2 + 128, c0:c0 + cw] = st_bf(f())
        for j in range(7):
          v = dst[j, r0 // 2:r0 // 2 + 128, c0:c0 + cw]
          deps += [pltpu.bitcast(v[r:r + 8, c:c + 128], F32)
                   for r in range(0, 128, 8) for c in range(0, cw, 128)]
    return deps

  def prep_from_value(m, dst):
    blk = [m[r:r + 256, c:c + 256] for r in (0, 256) for c in (0, 256)]
    for j, f in enumerate(beta_forms(*blk)):
      dst[j] = st_bf(f())

  def rows2(ref, r):
    return ref[pl.ds(r, H), :], ref[pl.ds(r + H, H), :]

  def init_quads(ref, r, cast=False):
    q = [ref[pl.ds(r + h, H), c:c + 256] for h in (0, H) for c in (0, 256)]
    return [v.astype(F32) for v in q] if cast else q

  def store_quads(ref, r, y):
    ref[pl.ds(r, H), :] = jnp.concatenate([y[0], y[1]], axis=1)
    ref[pl.ds(r + H, H), :] = jnp.concatenate([y[2], y[3]], axis=1)

  def ln_deps(ha, hb):
    return row_vregs(ha, 384) + row_vregs(hb, 384)

  class Body:
    def __init__(self):
      self.zm = zs[...] == 2
      self.q = []

    def take(self, n):
      n = max(n, 0)
      out = self.q[:n]
      del self.q[:n]
      return out

    def lhs_u(self, u, pri=(), cap=CAP):
      pri = list(pri)
      return ld_bf(tie(self.zm, u, interleave(pri, self.take(cap - len(pri))), True))

    def lhs_f(self, x, cap):
      return tie(self.zm, x, self.take(cap), False).astype(BF)

  def producer_thunks(bd, gam, get_u, rhs_fn, nt_dims, pri_of, order=AORD, nhf=2):
    def mk(k, j):
      def run():
        u = get_u(j)
        pri = pri_of(k)
        outs = []
        for hf in range(nhf):
          pp = pri[hf * len(pri) // nhf:(hf + 1) * len(pri) // nhf]
          lhs = bd.lhs_u(u(hf), pp)
          rhs = rhs_fn(j, hf)
          outs.append(dot_nt(lhs, rhs) if nt_dims else dot(lhs, rhs))
        gam.add(j, jnp.concatenate(outs, axis=1) if nhf > 1 else outs[0])
      return run
    return [mk(k, j) for k, j in enumerate(order)]

  def consumer_thunks(bd, gam, forms, rhs_fn, cap=0, order=BORD, cache=None):
    def mk(j):
      def run():
        if cache is not None and j in cache:
          lv = cache[j]
        else:
          lv = bd.lhs_f(forms[j](), cap)
          if cache is not None:
            cache[j] = lv
        gam.add(j, dot(lv, rhs_fn(j)))
      return run
    return [mk(j) for j in order]

  def pri_schedule(ts):
    done, out = set(), []
    for jb in BORD:
      new = [qq for qq in NEED[jb] if qq not in done]
      done.update(new)
      out.append([d for qq in new for d in ts[qq]])
    return lambda k: out[k]

  def scratch_u(j):
    return lambda hf: qa[j]

  def fresh_u(forms):
    def get(j):
      u = st_bf(forms[j]())
      qa[j] = u
      return lambda hf: u
    return get

  def run(thunks):
    for th in thunks:
      th()

  def ff_act(z):
    p = [half_silu(u) for u in z]
    ts = [row_vregs(jnp.maximum(jnp.maximum(u[:, 0:128], u[:, 128:256]),
                                jnp.maximum(u[:, 256:384], u[:, 384:512]))) for u in p]
    return p, pri_schedule(ts)

  def ff_a(bd, gz, get_u, cn, pri_of):
    return producer_thunks(bd, gz, get_u,
                           lambda j, hf: ld_bf(WA[j, :, cn * 512 + hf * 256:cn * 512 + hf * 256 + 256]),
                           False, pri_of)

  def ff_b(bd, gy, p, c):
    return consumer_thunks(bd, gy, alpha_forms(*p), lambda j: ld_bf(WB[j, c * 256:(c + 1) * 256, :]))

  def ff_step(bd, c, z, get_u, cn, gy):
    p, pri_of = ff_act(z)
    gz = Gamma()
    run(interleave(ff_a(bd, gz, get_u, cn, pri_of), ff_b(bd, gy, p, c)))
    return gz.result()

  def post_g(bd, t):
    r = pl.multiple_of(t * TM, TM)
    ga, gb_ = [ln_rows(v) for v in rows2(x1, r)]
    b = t // TPB
    rq_ = pl.multiple_of((t % TPB) * (H // 2), H // 2)
    for j, f in enumerate(alpha_forms(*quads(ga, gb_))):
      G[b, j, pl.ds(rq_, H // 2), :] = st_bf(f())
    for j in range(7):
      v = G[b, j, pl.ds(rq_, H // 2), :]
      bd.q.extend([pltpu.bitcast(v[r_:r_ + 8, c:c + 128], F32)
                   for r_ in range(0, H // 2, 8) for c in (0, 128)])

  def qp_thunks(bd, gq, t):
    b = t // TPB
    rn = pl.multiple_of((t % TPB) * (H // 2), H // 2)
    return producer_thunks(bd, gq, lambda j: (lambda hf: G[b, j, pl.ds(rn, H // 2), :]),
                           lambda j, hf: ld_bf(MQK[j]), False, lambda k: [], nhf=1)

  def s_thunks(bd, gs, get_u, b, c, pri_of):
    return producer_thunks(bd, gs, get_u,
                           lambda j, hf: ld_bf(G[b, j, c * 256 + hf * 128:c * 256 + (hf + 1) * 128, :]),
                           True, pri_of)

  class Att:
    def __init__(self):
      self.m = [None, None]
      self.l = [None, None]
      self.acc = None

  def soft(at, c, s):
    if c == 3:
      col = jax.lax.broadcasted_iota(jnp.int32, (H, 512), 1)
      s = [jnp.where(col < 512 - 48, u, NEG) for u in s]
    p, al, ts = [], [], []
    for hh in range(2):
      sa, sb = s[2 * hh], s[2 * hh + 1]
      mx = jnp.max(jnp.maximum(sa, sb), axis=-1, keepdims=True)
      mo = at.m[hh]
      mn = mx if mo is None else jnp.maximum(mo, mx)
      pa, pb = jnp.exp2(sa - mn), jnp.exp2(sb - mn)
      ta, tb = [(u[:, 0:128] + u[:, 128:256]) + (u[:, 256:384] + u[:, 384:512]) for u in (pa, pb)]
      if mo is None:
        a = None
        at.l[hh] = ta + tb
      else:
        a = jnp.exp2(mo - mn)
        at.l[hh] = at.l[hh] * a + (ta + tb)
      at.m[hh] = mn
      p += [pa, pb]
      al.append(a)
      ts += [row_vregs(ta), row_vregs(tb)]
    return p, al, pri_schedule(ts)

  def att_step(bd, at, b, c, s, get_u, bn_, cn):
    p, al, pri_of = soft(at, c, s)
    if at.acc is None:
      go = Gamma()
    else:
      go = Gamma([at.acc[0] * al[0], at.acc[1] * al[0], at.acc[2] * al[1], at.acc[3] * al[1]])
    pv = consumer_thunks(bd, go, alpha_forms(*p), lambda j: ld_bf(G[b, PVMAP[j], c * 256:(c + 1) * 256, :]))
    res = None
    if get_u is not None:
      gs = Gamma(transposed=True)
      run(interleave(s_thunks(bd, gs, get_u, bn_, cn, pri_of), pv))
      res = gs.result()
    else:
      run(pv)
    at.acc = go.result()
    if c < 3:
      bd.q[0:0] = row_vregs(at.l[0]) + row_vregs(at.l[1])
    return res

  def conv_unit(bd, U):
    start = (U % TPB) == 0
    ru = pl.multiple_of((U + 1) * TM, 8)
    rowi = jax.lax.broadcasted_iota(jnp.int32, (32, 128), 0)
    for l in range(4):
      ls = slice(l * 128, (l + 1) * 128)
      w = gb[:, ls]
      dwk = [DWB[k, :, ls] for k in range(KW)]
      we = w[0:32]
      wa = jnp.where(jnp.logical_and(start, rowi >= 16), 0.0, we)
      wb = jnp.where(jnp.logical_and(start, rowi < 16), 0.0, we)
      out = jnp.concatenate([conv_part(wa[0:24], 8, dwk), conv_part(wb[8:32], 8, dwk),
                             conv_part(w, TM, dwk)[16:]], axis=0)
      dc[pl.ds(ru, TM), ls] = out
      kk = jnp.where(U == 0, out[8:16], st[0:8, ls])
      st[0:8, ls] = kk
      d = dc[pl.ds(ru, TM), ls] - rep(kk, TM // 8, 0)
      d = jnp.concatenate([jnp.where(U == 0, 0.0, d[0:8]), d[8:]], axis=0)
      d2 = d * d
      st[8:16, ls] = st[8:16, ls] + jnp.sum(d.reshape(TM // 8, 8, 128), axis=0)
      st[16:24, ls] = st[16:24, ls] + jnp.sum(d2.reshape(TM // 8, 8, 128), axis=0)
      bd.q.extend(row_vregs(d2))

  def conv_part(win, nr, dwk):
    acc = [None, None]
    for rho in range(8):
      if rho == 0:
        tt = win[8:8 + nr] * rep(dwk[7], nr // 8, 0)
      else:
        u = (win[0:nr + 8] * rep(dwk[rho - 1], nr // 8 + 1, 0)
             + win[8:nr + 16] * rep(dwk[rho + 7], nr // 8 + 1, 0))
        tt = pltpu.roll(u, nr + 8 - rho, 0)[0:nr]
      acc[rho & 1] = tt if acc[rho & 1] is None else acc[rho & 1] + tt
    return acc[0] + acc[1]

  def conv_tail():
    rowi = jax.lax.broadcasted_iota(jnp.int32, (24, 128), 0)
    for l in range(4):
      ls = slice(l * 128, (l + 1) * 128)
      dwk = [DWB[k, :, ls] for k in range(KW)]
      halo = gb[TM:TM + 16, ls]
      w = jnp.concatenate([halo, jnp.zeros((8, 128), F32)], axis=0)
      out = conv_part(w, 8, dwk)
      dc[N + TM:N + TM + 8, ls] = out
      d = out - st[0:8, ls]
      st[8:16, ls] = st[8:16, ls] + d
      st[16:24, ls] = st[16:24, ls] + d * d
    del rowi

  def epi_mvo(bd, t, cap=0):
    r = pl.multiple_of(t * TM, TM)
    rl = [1.0 / jnp.sum(lsc[hh], axis=-1, keepdims=True) for hh in range(2)]
    oq = [osc[0] * rl[0], osc[1] * rl[0], osc[2] * rl[1], osc[3] * rl[1]]
    g = Gamma(init_quads(x1, r))
    run(consumer_thunks(bd, g, alpha_forms(*oq), lambda j: ld_bf(MVO[j]), cap=cap))
    store_quads(x1, r, g.result())
    return [ln_rows(v) for v in rows2(x1, r)]

  def epi_pw1(bd, ha, hb, sl, cache):
    g = Gamma()
    run(consumer_thunks(bd, g, alpha_forms(*quads(ha, hb)),
                        lambda j: ld_bf(WP1[j, :, sl * 256:(sl + 1) * 256]), order=AORD, cache=cache))
    a1, b1, a2, b2 = g.result()
    gb[16:16 + H, sl * 256:(sl + 1) * 256] = a1 + a1 * jnp.tanh(b1)
    gb[16 + H:16 + TM, sl * 256:(sl + 1) * 256] = a2 + a2 * jnp.tanh(b2)
    return [gb[r:r + 8, c:c + 128] for r in range(16, 16 + TM, 8) for c in (sl * 256, sl * 256 + 128)]

  def pre3(bd, t):
    r = pl.multiple_of(t * TM, TM)
    mu = rep(bn[0:8, :], H // 8, 0)
    hrs = rep(bn[8:16, :], H // 8, 0)
    hs = [half_silu((dc[pl.ds(r + TM + 8 + h, H), :] - mu) * hrs) for h in (0, H)]
    g = Gamma(init_quads(x1, r))
    run(consumer_thunks(bd, g, alpha_forms(*quads(*hs)), lambda j: ld_bf(WP2[j])))
    store_quads(x1, r, g.result())
    ha, hb = [ln_rows(v) for v in rows2(x1, r)]
    return ha, hb

  def post3(bd, t):
    r = pl.multiple_of(t * TM, TM)
    for h, v in zip((0, H), rows2(x1, r)):
      xo[pl.ds(r + h, H), :] = ln_rows(v).astype(BF)
    ol = xo[pl.ds(r, TM), :].astype(F32)
    bd.q.extend([ol[r_:r_ + 8, 384:512] for r_ in range(0, TM, 16)])

  for j in range(7):
    for b in range(NB):
      G[b, j, T // 4:1024, :] = jnp.zeros((1024 - T // 4, 256), U32)
  gb[...] = jnp.zeros(gb.shape, F32)
  st[...] = jnp.zeros(st.shape, F32)
  x1[0:TM, :] = jnp.zeros((TM, D), F32)

  xcopy(0).wait()
  zs[...] = pltpu.bitcast(xo[0:16, 0:128], U32) >> 31
  wcopy(I_A1).wait()
  prep_weight(ra1, WA, 256, 1024, 0.5)
  bd = Body()
  ha, hb = [ln_rows(v.astype(F32)) for v in rows2(xo, 0)]
  wcopy(I_B1).wait()
  bd.q.extend(prep_weight(rb1, WB, 1024, 256, 0.5))
  gz = Gamma()
  run(ff_a(bd, gz, fresh_u(alpha_forms(*quads(ha, hb))), 0, lambda k: []))
  for k, v in enumerate(gz.result()):
    sS[k] = v
  for i in (I_Q, I_K, I_V, I_O):
    wcopy(i).wait()
  prep_from_value(dot_nt(rq[...], rk[...]) * QSCALE, MQK)
  prep_from_value(dot(rv[...], ro[...]), MVO)

  def p1_body(t, last):
    bd = Body()
    r0 = pl.multiple_of(t * TM, TM)
    if not last:
      xcopy(t + 1).wait()
      rn = pl.multiple_of((t + 1) * TM, TM)
      ha, hb = [ln_rows(v.astype(F32)) for v in rows2(xo, rn)]
      bd.q.extend(ln_deps(ha, hb))
    post_g(bd, jnp.maximum(t - 1, 0))
    gy = Gamma(init_quads(xo, r0, cast=True))
    z = ff_step(bd, 0, [sS[k] for k in range(4)], scratch_u, 1, gy)
    if not last:
      z = ff_step(bd, 1, z, fresh_u(alpha_forms(*quads(ha, hb))), 0, gy)
      store_quads(x1, r0, gy.result())
      for k in range(4):
        sS[k] = z[k]
    else:
      p, pri_of = ff_act(z)
      bth = ff_b(bd, gy, p, 1)
      gq = Gamma()
      run(merge(qp_thunks(bd, gq, 0), bth[:3]))
      gs = Gamma(transposed=True)
      run(merge(s_thunks(bd, gs, fresh_u(phi_forms(*gq.result())), 0, 0, lambda k: []), bth[3:]))
      store_quads(x1, r0, gy.result())
      for k, v in enumerate(gs.result()):
        sS[k] = v

  jax.lax.fori_loop(0, NT - 1, lambda t, c: (p1_body(t, False), c)[1], 0)
  p1_body(NT - 1, True)

  def p2_body(i, first, last):
    bd = Body()
    b = i // TPB
    bn_ = (i + 1) // TPB
    at = Att()
    if first:
      for k in (I_P1, I_DW, I_P2, I_A2, I_B2):
        wcopy(k).wait()
      post_g(bd, NT - 1)
      dwf = rdw[...].astype(F32)
      for k in range(KW):
        DWB[k] = jnp.broadcast_to(dwf[k:k + 1, :], (8, D))
      bd.q.extend(prep_weight(rp1, WP1, 256, 512, 0.5))
      bd.q.extend(prep_weight(rp2, WP2, 256, 256, 1.0))
      bd.q.extend(prep_weight(ra2, WA, 256, 1024, 0.5))
      bd.q.extend(prep_weight(rb2, WB, 1024, 256, 0.5))
    else:
      conv_unit(bd, i - 2)
      halo = gb[TM:TM + 16, :]
    s = [sS[k] for k in range(4)]
    s = att_step(bd, at, b, 0, s, scratch_u, b, 1)
    if not first:
      ha, hb = epi_mvo(bd, i - 1)
    s = att_step(bd, at, b, 1, s, scratch_u, b, 2)
    if not first:
      bd.q.extend(ln_deps(ha, hb))
    s = att_step(bd, at, b, 2, s, scratch_u, b, 3)
    if not first:
      cache = {}
      gd = epi_pw1(bd, ha, hb, 0, cache)
      gb[0:16, :] = halo
      gd += epi_pw1(bd, ha, hb, 1, cache)
      bd.q.extend(gd)
    if not last:
      gq = Gamma()
      run(qp_thunks(bd, gq, i + 1))
      s = att_step(bd, at, b, 3, s, fresh_u(phi_forms(*gq.result())), bn_, 0)
      for k in range(4):
        sS[k] = s[k]
    else:
      att_step(bd, at, b, 3, s, None, None, None)
    for k in range(4):
      osc[k] = at.acc[k]
    for hh in range(2):
      lsc[hh] = at.l[hh]

  p2_body(0, True, False)
  jax.lax.fori_loop(1, NT - 1, lambda i, c: (p2_body(i, False, False), c)[1], 0)
  p2_body(NT - 1, False, True)

  bd = Body()
  conv_unit(bd, NT - 2)
  halo = gb[TM:TM + 16, :]
  ha, hb = epi_mvo(bd, NT - 1, cap=2 * CAP)
  cache = {}
  epi_pw1(bd, ha, hb, 0, cache)
  gb[0:16, :] = halo
  epi_pw1(bd, ha, hb, 1, cache)
  conv_unit(bd, NT - 1)
  conv_tail()
  n_s = N // 8
  s1 = st[8:16, :]
  mu_s = st[0:8, :] + s1 * (1.0 / n_s)
  m2_s = st[16:24, :] - s1 * s1 * (1.0 / n_s)
  mu = jnp.sum(mu_s, axis=0, keepdims=True) * 0.125
  dm = mu_s - mu
  var = jnp.sum(m2_s + dm * dm * n_s, axis=0, keepdims=True) * (1.0 / N)
  bn[0:8, :] = jnp.broadcast_to(mu, (8, D))
  bn[8:16, :] = jnp.broadcast_to(0.5 * jax.lax.rsqrt(var + EPS), (8, D))

  bd = Body()
  ha, hb = pre3(bd, 0)
  gz = Gamma()
  run(ff_a(bd, gz, fresh_u(alpha_forms(*quads(ha, hb))), 0, lambda k: []))
  for k, v in enumerate(gz.result()):
    sS[k] = v

  def p3_body(t, last):
    bd = Body()
    r0 = pl.multiple_of(t * TM, TM)

    @pl.when(t >= 2)
    def _():
      ocopy(t - 2).start()

    post3(bd, jnp.maximum(t - 1, 0))
    if not last:
      ha, hb = pre3(bd, t + 1)
      bd.q[0:0] = ln_deps(ha, hb)
    gy = Gamma(init_quads(x1, r0))
    z = ff_step(bd, 0, [sS[k] for k in range(4)], scratch_u, 1, gy)
    if not last:
      z = ff_step(bd, 1, z, fresh_u(alpha_forms(*quads(ha, hb))), 0, gy)
      for k in range(4):
        sS[k] = z[k]
    else:
      p, _ = ff_act(z)
      run(ff_b(bd, gy, p, 1))
    store_quads(x1, r0, gy.result())

  jax.lax.fori_loop(0, NT - 1, lambda t, c: (p3_body(t, False), c)[1], 0)
  p3_body(NT - 1, True)

  bd = Body()
  ocopy(NT - 2).start()
  post3(bd, NT - 1)
  ocopy(NT - 1).start()
  for t in range(NT):
    ocopy(t).wait()


@jax.jit
def pallas_standalone__conformer_family_conformer__speech_kernel(
    x, w_ff1_a, w_ff1_b, w_q, w_k, w_v, w_o, w_pw1, dw, w_pw2, w_ff2_a, w_ff2_b):
  hbm = pl.BlockSpec(memory_space=pl.ANY)
  V = pltpu.VMEM
  out = pl.pallas_call(
      kernel,
      out_shape=jax.ShapeDtypeStruct((N, D), x.dtype),
      in_specs=[hbm] * 12,
      out_specs=hbm,
      scratch_shapes=[
          V((N, D), BF),
          V((D, FH), BF), V((FH, D), BF), V((D, FH), BF), V((FH, D), BF),
          V((D, D), BF), V((D, D), BF), V((D, D), BF), V((D, D), BF),
          V((D, 2 * D), BF), V((KW, D), BF), V((D, D), BF),
          V((7, 128, 1024), U32), V((7, 512, 256), U32),
          V((7, 128, 256), U32), V((7, 128, 256), U32),
          V((7, 128, 512), U32), V((7, 128, 256), U32),
          V((KW, 8, D), F32),
          V((N, D), F32),
          V((N + TM + 8, D), F32),
          V((NB, 7, 1024, 256), U32),
          V((TM + 16, D), F32),
          V((4, H, 512), F32),
          V((7, H // 2, 256), U32),
          V((4, H, 256), F32),
          V((2, H, 128), F32),
          V((24, D), F32), V((16, D), F32), V((8, 128), U32),
          pltpu.SemaphoreType.DMA((2 * NT + 11,)),
      ],
      compiler_params=pltpu.CompilerParams(vmem_limit_bytes=124 * 1024 * 1024),
  )(x.reshape(N, D), w_ff1_a, w_ff1_b, w_q, w_k, w_v, w_o, w_pw1, dw, w_pw2, w_ff2_a, w_ff2_b)
  return out.reshape(NB, T, D)
```

```python
import jax
import jax.numpy as jnp
import jax.experimental.pallas as pl
import jax.experimental.pallas.tpu as pltpu

BF = jnp.bfloat16
F32 = jnp.float32
U32 = jnp.uint32

NB, T, D, FH, KW = 2, 4000, 512, 2048, 15
N = NB * T
TM = 800
H = TM // 2
NT = N // TM
TPB = T // TM
EPS = 1e-5
QSCALE = D ** -0.5 * 1.4426950408889634
NEG = -1e30

PVMAP = [0, 2, 6, 5, 3, 4, 1]
AORD = [0, 3, 4, 6, 2, 1, 5]
TORD = [0, 3, 4, 6, 1, 2, 5]
BORD = [2, 4, 0, 3, 6, 5, 1]
W_LN, W_PREP = 36, 9
BUD1, BUD2, BUD3, BUDM = 500, 700, 620, 700
NHI1, NHI2, NHI3 = 25, 40, 30
NHI, NHIF, HIW, GATE, NG = 40, 0, 1, 2, 6
P3POS = 6
BUDL, BUDL2, BUDL3 = 1500, 850, 850
FLD = 2
BUDP = 850
HOSTL = (0,)
HOST8 = (0, 1, 2)
DEBUG = False
W_CONV = 36
BUDGET = 560
PHASES = ('P1', 'P1L', 'P2F', 'P2', 'P2L', 'P3', 'P3L')
CONTRIB = [((0, 1), (3, 1)), ((2, 1), (3, -1)), ((1, 1), (3, 1)), ((0, 1), (2, 1)),
           ((0, -1), (1, 1)), ((3, 1),), ((0, 1),)]


def dot(a, b):
  return jnp.dot(a, b, preferred_element_type=F32)


def dot_nt(a, b):
  return jax.lax.dot_general(a, b, (((1,), (1,)), ((), ())), preferred_element_type=F32)


def alpha_forms(a11, a12, a21, a22):
  return [lambda: a11 + a22, lambda: a21 + a22, lambda: a11, lambda: a22,
          lambda: a11 + a12, lambda: a21 - a11, lambda: a12 - a22]


def beta_forms(b11, b12, b21, b22):
  return [lambda: b11 + b22, lambda: b11, lambda: b12 - b22, lambda: b21 - b11,
          lambda: b22, lambda: b11 + b12, lambda: b21 + b22]


def phi_forms(q11, q12, q21, q22):
  return beta_forms(q11, q21, q12, q22)


def quads(ha, hb):
  return ha[:, :256], ha[:, 256:], hb[:, :256], hb[:, 256:]


class Gamma:
  def __init__(self, init=None, transposed=False, on_final=None, reps=1):
    self.p = [None] * 4 if init is None else list(init)
    self.sg = [1] * 4
    self.left = [4 * reps, 2 * reps, 2 * reps, 4 * reps]
    self.tr = transposed
    self.on_final = on_final

  def add(self, j, m):
    for q, sg in CONTRIB[j]:
      if self.tr and q in (1, 2):
        q = 3 - q
      v = self.p[q]
      if callable(v):
        v = v()
      s = self.sg[q]
      if v is None:
        self.p[q], self.sg[q] = m, sg
      elif s == 1:
        self.p[q] = v + m if sg == 1 else v - m
      else:
        self.p[q], self.sg[q] = (m - v, 1) if sg == 1 else (v + m, -1)
      self.left[q] -= 1
      if self.left[q] == 0:
        assert self.sg[q] == 1
        if self.on_final is not None:
          self.on_final(q, self.p[q])

  def result(self):
    assert all(n == 0 for n in self.left)
    return list(self.p)


def rep(x, n, axis):
  return jnp.concatenate([x] * n, axis=axis) if n > 1 else x


def ld_bf(u):
  return pltpu.bitcast(u, BF)


def st_bf(x):
  return pltpu.bitcast(x.astype(BF), U32)


def ln_rows(x):
  m = jnp.mean(x, axis=-1, keepdims=True)
  xc = x - m
  v = jnp.mean(xc * xc, axis=-1, keepdims=True)
  return xc * jax.lax.rsqrt(v + EPS)


def half_silu(hz):
  return hz + hz * jnp.tanh(hz)


def row_vregs(x, c0=0):
  return [x[r:r + 8, c0:c0 + 128] for r in range(0, x.shape[0], 8)]


def tie(zm, u, deps, cast):
  if not deps:
    return u
  n = u.shape[0] // 8
  nk = u.shape[1] // 128
  slots = n * nk
  assign = {}
  for idx, d in enumerate(deps):
    assign[(idx * slots) // len(deps)] = d
  rows = []
  for rb in range(n):
    blk = u[rb * 8:(rb + 1) * 8]
    if any((rb * nk + k) in assign for k in range(nk)):
      parts = []
      for k in range(nk):
        pc = blk[:, k * 128:(k + 1) * 128]
        d = assign.get(rb * nk + k)
        if d is not None:
          pc = jnp.where(zm, pltpu.bitcast(d, U32) if cast else d, pc)
        parts.append(pc)
      blk = jnp.concatenate(parts, axis=1)
    rows.append(blk)
  return jnp.concatenate(rows, axis=0)


def sel(c, a, b):
  if isinstance(c, bool):
    return a if c else b
  return jnp.where(c, a, b)


def mult(x, n):
  return x if isinstance(x, int) else pl.multiple_of(x, n)


def interleave(a, b):
  out = []
  for i in range(max(len(a), len(b))):
    if i < len(a):
      out.append(a[i])
    if i < len(b):
      out.append(b[i])
  return out


def merge(s1, s2):
  out, n1, n2, i, j = [], len(s1), len(s2), 0, 0
  while i < n1 or j < n2:
    if j >= n2 or (i < n1 and i * n2 <= j * n1):
      out.append(s1[i]); i += 1
    else:
      out.append(s2[j]); j += 1
  return out


def kernel(z_s, x_h, wa1_h, wb1_h, wq_h, wk_h, wv_h, wo_h, wp1_h, dw_h, wp2_h, wa2_h, wb2_h, out_h,
           xo, ra1, rb1, ra2, rb2, rq, rk, rv, ro, rp1, rdw, rp2,
           WA, WB, MQK, MVO, WP1, WP2, DWB, x1, dc, G, gb, sS, qa, osc, lsc, st, bn, zs, sem):

  def xcopy(t):
    return pltpu.make_async_copy(x_h.at[pl.ds(t * TM, TM)], xo.at[pl.ds(t * TM, TM)], sem.at[t])

  def ocopy(t):
    return pltpu.make_async_copy(xo.at[pl.ds(t * TM, TM)], out_h.at[pl.ds(t * TM, TM)], sem.at[NT + 11 + t])

  wsrc = [wa1_h, wb1_h, wq_h, wk_h, wv_h, wo_h, wp1_h, dw_h, wp2_h, wa2_h, wb2_h]
  wdst = [ra1, rb1, rq, rk, rv, ro, rp1, rdw, rp2, ra2, rb2]
  I_A1, I_B1, I_Q, I_K, I_V, I_O, I_P1, I_DW, I_P2, I_A2, I_B2 = range(11)

  def wcopy(i):
    return pltpu.make_async_copy(wsrc[i], wdst[i], sem.at[NT + i])

  xcopy(0).start()
  wcopy(I_A1).start()
  wcopy(I_B1).start()
  xcopy(1).start()
  for i in (I_Q, I_K, I_V, I_O):
    wcopy(i).start()
  for t in range(2, NT):
    xcopy(t).start()
  for i in (I_P1, I_DW, I_P2, I_A2, I_B2):
    wcopy(i).start()

  def prep_weight(raw, dst, kh, nh, scale, cw=256):
    deps = []
    for c0 in range(0, nh, cw):
      for r0 in range(0, kh, 256):
        blk = [raw[r:r + 256, c:c + cw].astype(F32) * scale
               for r in (r0, kh + r0) for c in (c0, nh + c0)]
        for j, f in enumerate(beta_forms(*blk)):
          dst[j, r0 // 2:r0 // 2 + 128, c0:c0 + cw] = st_bf(f())
        for j in range(7):
          v = dst[j, r0 // 2:r0 // 2 + 128, c0:c0 + cw]
          deps += [pltpu.bitcast(v[r:r + 8, c:c + 128], F32)
                   for r in range(0, 128, 8) for c in range(0, cw, 128)]
    return deps

  def prep_from_value(m, dst):
    blk = [m[r:r + 256, c:c + 256] for r in (0, 256) for c in (0, 256)]
    for j, f in enumerate(beta_forms(*blk)):
      dst[j] = st_bf(f())

  def rows2(ref, r):
    return ref[pl.ds(r, H), :], ref[pl.ds(r + H, H), :]

  def init_quads(ref, r, cast=False):
    q = [ref[pl.ds(r + h, H), c:c + 256] for h in (0, H) for c in (0, 256)]
    return [v.astype(F32) for v in q] if cast else q

  def store_quads(ref, r, y):
    ref[pl.ds(r, H), :] = jnp.concatenate([y[0], y[1]], axis=1)
    ref[pl.ds(r + H, H), :] = jnp.concatenate([y[2], y[3]], axis=1)

  def store_tied(bd, ref, lead, r0, c0, val, step):
    for rr in range(0, val.shape[0], step):
      n = min(step, val.shape[0] - rr)
      ref[lead + (pl.ds(r0 + rr, n), slice(c0, c0 + val.shape[1]))] = val[rr:rr + n]
      got = ref[lead + (pl.ds(r0 + rr + n - 8, 8), slice(c0, c0 + 128))]
      bd.push([got if got.dtype == F32 else pltpu.bitcast(got, F32)], n * val.shape[1] // 1024)

  def ln_deps(ha, hb):
    return row_vregs(ha, 384) + row_vregs(hb, 384)

  class Body:
    def __init__(self, budget=BUDGET, nhi=25):
      self.nhi = nhi
      self.zm = zs[...] == 2
      self.budget = budget
      self.hi = []
      self.lo = []
      self.anchors = []

    def push(self, deps, w, hi=False):
      (self.hi if hi else self.lo).extend((w, 1, (lambda a, d=d: [d])) for d in deps)

    def push_lazy(self, w, n, fn):
      self.lo.append((w, n, fn))

    def note_result(self, r):
      self.anchors.append(r[0:8, 0:128])

    def gate(self, x, anchor):
      return jnp.where(self.zm, anchor, x)

    def anchor(self):
      return self.anchors[-GATE] if GATE and len(self.anchors) >= GATE else None

    def take(self, budget, nhi, slots=50):
      out, tot = [], 0
      anchor = self.anchor()
      while self.hi and len(out) < nhi:
        w, n, fn = self.hi.pop(0)
        out += fn(anchor)
        tot += w * HIW
      while self.lo:
        w, n, fn = self.lo[0]
        if tot + w > budget or len(out) + n > slots:
          break
        self.lo.pop(0)
        tot += w
        out += fn(anchor)
      return out

    def flush_lo(self):
      anchor = self.anchor()
      rest = []
      for w, n, fn in self.lo:
        ds = fn(anchor)
        rest += [(w // max(n, 1), 1, (lambda a, d=d: [d])) for d in ds]
      self.lo = rest

    def flush(self):
      chain = [self.anchor()]
      for _, n, fn in self.hi + self.lo:
        out = fn(chain[-FLD] if len(chain) >= FLD else chain[0])
        if n > 1:
          chain.append(out[0])
      self.hi, self.lo = [], []

    def lhs_u(self, u, budget):
      return ld_bf(tie(self.zm, u, self.take(budget, self.nhi), True))

    def lhs_f(self, x, budget):
      return tie(self.zm, x, self.take(budget, NHIF if budget else 0, 2 * (x.shape[0] // 8)), False).astype(BF)

  def producer_thunks(bd, gam, get_u, rhs_fn, nt_dims, order=AORD, nhf=2):
    def mk(j):
      def run_():
        u = get_u(j)
        outs = []
        for hf in range(nhf):
          lhs = bd.lhs_u(u(hf), bd.budget)
          rhs = rhs_fn(j, hf)
          outs.append(dot_nt(lhs, rhs) if nt_dims else dot(lhs, rhs))
          bd.note_result(outs[-1])
        gam.add(j, jnp.concatenate(outs, axis=1) if nhf > 1 else outs[0])
      return run_
    return [mk(j) for j in order]

  def consumer_thunks(bd, gam, forms, rhs_fn, budget=0, order=BORD, cache=None):
    def mk(j):
      def run_():
        if cache is not None and j in cache:
          lv = cache[j]
        else:
          lv = bd.lhs_f(forms[j](), budget)
          if cache is not None:
            cache[j] = lv
        res = dot(lv, rhs_fn(j))
        bd.note_result(res)
        gam.add(j, res)
      return run_
    return [mk(j) for j in order]

  def scratch_u(j):
    return lambda hf: qa[j]

  def fresh_u(forms):
    def get(j):
      u = st_bf(forms[j]())
      qa[j] = u
      return lambda hf: u if hf == 0 else qa[j]
    return get

  def run(thunks):
    for th in thunks:
      th()

  def ff_act(bd, p, skip=()):
    def cb(q, z):
      if q in skip:
        p[q] = z
        return
      u = half_silu(z)
      p[q] = u
      bd.push(row_vregs(jnp.maximum(jnp.maximum(u[:, 0:128], u[:, 128:256]),
                                    jnp.maximum(u[:, 256:384], u[:, 384:512]))), 20, hi=True)
    return cb

  def ff_carried(bd):
    p = [sS[0], sS[1], sS[2], None]
    ff_act(bd, p)(3, sS[3])
    return p

  def ff_a(bd, gz, get_u, cn):
    return producer_thunks(bd, gz, get_u,
                           lambda j, hf: ld_bf(WA[j, :, cn * 512 + hf * 256:cn * 512 + hf * 256 + 256]), False)

  def ff_b(bd, gy, p, c):
    return consumer_thunks(bd, gy, alpha_forms(*p), lambda j: ld_bf(WB[j, c * 256:(c + 1) * 256, :]))

  def ff_step(bd, c, p, get_u, cn, gy, act, extra=None):
    pn = [None] * 4
    gz = Gamma(on_final=ff_act(bd, pn, () if act else (3,)))
    seq = interleave(ff_a(bd, gz, get_u, cn), ff_b(bd, gy, p, c))
    if extra is not None:
      seq[extra[0]:extra[0]] = extra[1]
    run(seq)
    return pn

  def post_g(bd, t):
    r = mult(t * TM, TM)
    ga, gb_ = [ln_rows(v) for v in rows2(x1, r)]
    bd.push(ln_deps(ga, gb_), W_LN)
    b = t // TPB
    rq_ = mult((t % TPB) * (H // 2), H // 2)
    for j, f in enumerate(alpha_forms(*quads(ga, gb_))):
      v = st_bf(f())
      vd = [pltpu.bitcast(v[r_:r_ + 8, 128:256], F32) for r_ in range(0, H // 2, 8)]
      for r_ in range(0, H // 2, 40):
        bd.push(vd[r_ // 8:(r_ + 40) // 8], 16)
        if r_ + 40 in (120, 200):
          lo_ = 0 if r_ + 40 == 120 else 120
          store_tied(bd, G, (b, j), rq_ + lo_, 0, v[lo_:r_ + 40], 200)

  def qp_thunks(bd, gq, t):
    b = t // TPB
    rn = mult((t % TPB) * (H // 2), H // 2)
    return producer_thunks(bd, gq, lambda j: (lambda hf: G[b, j, pl.ds(rn, H // 2), :]),
                           lambda j, hf: ld_bf(MQK[j]), False, nhf=1)

  def s_thunks(bd, gs, get_u, b, c):
    return producer_thunks(bd, gs, get_u,
                           lambda j, hf: ld_bf(G[b, j, c * 256 + hf * 128:c * 256 + (hf + 1) * 128, :]),
                           True, order=TORD)

  class Att:
    def __init__(self):
      self.m = [None, None]
      self.l = [None, None]
      self.al = [None, None]
      self.acc = None

  def soft_cb(bd, at, c, p):
    held = {}

    def cb(q, sv):
      if c == 3:
        col = jax.lax.broadcasted_iota(jnp.int32, (H, 512), 1)
        sv = jnp.where(col < 512 - 48, sv, NEG)
      if q in (0, 2):
        held[q] = sv
        return
      hh = q // 2
      sa, sb = held[q - 1], sv
      mx = jnp.max(jnp.maximum(sa, sb), axis=-1, keepdims=True)
      mo = at.m[hh]
      mn = mx if mo is None else jnp.maximum(mo, mx)
      pa, pb = jnp.exp2(sa - mn), jnp.exp2(sb - mn)
      ta, tb = [(u[:, 0:128] + u[:, 128:256]) + (u[:, 256:384] + u[:, 384:512]) for u in (pa, pb)]
      if mo is None:
        at.al[hh] = None
        at.l[hh] = ta + tb
      else:
        at.al[hh] = jnp.exp2(mo - mn)
        at.l[hh] = at.l[hh] * at.al[hh] + (ta + tb)
      at.m[hh] = mn
      p[q - 1], p[q] = pa, pb
      for t_ in ((ta, tb) if hh == 0 else (tb, ta)):
        bd.push(row_vregs(t_), 12, hi=True)
      if c < 3:
        bd.push(row_vregs(at.l[hh]), 4, hi=True)
    return cb

  def att_carried(bd, at):
    p = [None] * 4
    cb = soft_cb(bd, at, 0, p)
    for q in range(4):
      cb(q, sS[q])
    return p

  def att_step(bd, at, b, c, p, get_u, bn_, cn, act=True, pv_budget=0):
    if at.acc is None:
      go = Gamma()
    else:
      acc = at.acc
      go = Gamma([(lambda q=q: acc[q] * al[q // 2]) for q in range(4)])
    al = list(at.al)
    pv = consumer_thunks(bd, go, alpha_forms(*p), lambda j: ld_bf(G[b, PVMAP[j], c * 256:(c + 1) * 256, :]),
                         budget=pv_budget)
    res = None
    if get_u is not None:
      pn = [None] * 4
      gs = Gamma(transposed=True, on_final=soft_cb(bd, at, cn, pn) if act else None)
      run(interleave(s_thunks(bd, gs, get_u, bn_, cn), pv))
      res = pn if act else gs.result()
    else:
      run(pv)
    at.acc = go.result()
    return res

  LS = TM // 8

  def conv_outputs(U, ls, dwk, u0, u1):
    start = (U % TPB) == 0
    win = {}

    def inp(u):
      if u not in win:
        win[u] = gb[ls, pl.ds(8 + u, 8, stride=LS), :]
      return win[u]

    outs = []
    for u in range(u0, u1):
      acc = [None, None]
      for k in range(KW):
        ui = u + k - KW // 2
        v = inp(ui)
        if start and u < 15 and ((u < 8) != (ui < 8)):
          v = jnp.where(sub0, 0.0, v)
        t = v * dwk[k]
        acc[k & 1] = t if acc[k & 1] is None else acc[k & 1] + t
      outs.append(acc[0] + acc[1])
    return outs

  def conv_unit(bd, U, lanes=(0, 1, 2, 3)):
    ru = (U + 1) * TM
    bounds = [(LS * g + NG // 2) // NG for g in range(NG + 1)]

    def make(l):
      ls = slice(l * 128, (l + 1) * 128)
      state = {}

      def group(g, anchor):
        u0, u1 = bounds[g], bounds[g + 1]
        dwk = [DWB[k, :, ls] for k in range(KW)]
        if anchor is not None:
          dwk = [bd.gate(v, anchor) for v in dwk]
        outs = conv_outputs(U, l, dwk, u0, u1)
        if g == 0:
          if U == 0:
            st[0:8, ls] = outs[8]
          state["k"] = outs[8] if U == 0 else st[0:8, ls]
          state["s1"] = st[8:16, ls]
          state["s2"] = st[16:24, ls]
        deps = []
        for u, o in zip(range(u0, u1), outs):
          d = o - state["k"]
          if U == 0 and u < 8:
            d = jnp.where(sub0, 0.0, d)
          d2 = d * d
          state["s1"] = state["s1"] + d
          state["s2"] = state["s2"] + d2
          dc[l, pl.ds(ru + u, 8, stride=LS), :] = o
          deps.append(d2)
        deps.append(dc[l, pl.ds(ru + u1 - 1, 8, stride=LS), :])
        if g == NG - 1:
          st[8:16, ls] = state["s1"]
          st[16:24, ls] = state["s2"]
        return deps
      return group

    for l in lanes:
      grp = make(l)
      for g in range(NG):
        n = bounds[g + 1] - bounds[g]
        bd.push_lazy(W_CONV * n + 15, n + 1, lambda a, grp=grp, g=g: grp(g, a))

  def conv_part(win, nr, dwk):
    acc = [None, None]
    for rho in range(8):
      if rho == 0:
        tt = win[8:8 + nr] * rep(dwk[7], nr // 8, 0)
      else:
        u = (win[0:nr + 8] * rep(dwk[rho - 1], nr // 8 + 1, 0)
             + win[8:nr + 16] * rep(dwk[rho + 7], nr // 8 + 1, 0))
        tt = pltpu.roll(u, nr + 8 - rho, 0)[0:nr]
      acc[rho & 1] = tt if acc[rho & 1] is None else acc[rho & 1] + tt
    return acc[0] + acc[1]

  def conv_exposed(bd, U, lanes):
    keep = bd.hi, bd.lo
    bd.hi, bd.lo = [], []
    conv_unit(bd, U, lanes)
    for _, _, fn in bd.lo:
      fn(None)
    bd.hi, bd.lo = keep

  def conv_tail(lanes):
    for l in lanes:
      ls = slice(l * 128, (l + 1) * 128)
      dwk = [DWB[k, :, ls] for k in range(KW)]
      halo = gb[l, TM:TM + 16, :]
      w = jnp.concatenate([halo, jnp.zeros((8, 128), F32)], axis=0)
      out = conv_part(w, 8, dwk)
      dc[l, N + TM:N + TM + 8, :] = out
      d = out - st[0:8, ls]
      st[8:16, ls] = st[8:16, ls] + d
      st[16:24, ls] = st[16:24, ls] + d * d

  def epi_mvo(bd, t, budget=0):
    r = mult(t * TM, TM)
    rl = [1.0 / jnp.sum(lsc[hh], axis=-1, keepdims=True) for hh in range(2)]
    oq = [osc[0] * rl[0], osc[1] * rl[0], osc[2] * rl[1], osc[3] * rl[1]]
    g = Gamma(init_quads(x1, r))
    run(consumer_thunks(bd, g, alpha_forms(*oq), lambda j: ld_bf(MVO[j]), budget=budget))
    y = g.result()
    xs = [jnp.concatenate([y[0], y[1]], axis=1), jnp.concatenate([y[2], y[3]], axis=1)]
    for h, v in zip((0, H), xs):
      store_tied(bd, x1, (), r + h, 0, v, 80)
    return [ln_rows(v) for v in xs]

  def epi_pw1(bd, ha, hb, sl, cache, budget=0, pre_store=None):
    g = Gamma()
    run(consumer_thunks(bd, g, alpha_forms(*quads(ha, hb)),
                        lambda j: ld_bf(WP1[j, :, sl * 256:(sl + 1) * 256]), order=AORD, cache=cache,
                        budget=budget))
    if pre_store is not None:
      pre_store()
    a1, b1, a2, b2 = g.result()
    deps = []
    for h, gv in ((0, a1 + a1 * jnp.tanh(b1)), (H, a2 + a2 * jnp.tanh(b2))):
      for k in range(2):
        gb[2 * sl + k, 16 + h:16 + h + H, :] = gv[:, k * 128:(k + 1) * 128]
        deps += [gb[2 * sl + k, r:r + 8, :] for r in range(16 + h, 16 + h + H, 8)]
    return deps

  def pre3(bd, t):
    r = mult(t * TM, TM)
    mu = rep(bn[0:8, :], H // 8, 0)
    hrs = rep(bn[8:16, :], H // 8, 0)
    hs = [half_silu((jnp.concatenate([dc[l, pl.ds(r + TM + 8 + h, H), :] for l in range(4)], axis=1)
                     - mu) * hrs) for h in (0, H)]
    for u in hs:
      bd.push(row_vregs(jnp.maximum(jnp.maximum(u[:, 0:128], u[:, 128:256]),
                                    jnp.maximum(u[:, 256:384], u[:, 384:512]))), 24, hi=True)
    g = Gamma(init_quads(x1, r))
    holder = []

    def finish():
      y = g.result()
      xs = [jnp.concatenate([y[0], y[1]], axis=1), jnp.concatenate([y[2], y[3]], axis=1)]
      ha, hb = [ln_rows(v) for v in xs]
      bd.lo[0:0] = [(W_LN, 1, (lambda a, d=d: [d])) for d in ln_deps(ha, hb)]
      for h, v in zip((0, H), xs):
        store_tied(bd, x1, (), r + h, 0, v, 80)
      holder.extend([ha, hb])

    return consumer_thunks(bd, g, alpha_forms(*quads(*hs)), lambda j: ld_bf(WP2[j])) + [finish], holder

  def post3(bd, t):
    r = mult(t * TM, TM)
    for h, v in zip((0, H), rows2(x1, r)):
      xo[pl.ds(r + h, H), :] = ln_rows(v).astype(BF)
    ol = xo[pl.ds(r, TM), :].astype(F32)
    bd.push([ol[r_:r_ + 8, 384:512] for r_ in range(0, TM, 16)], 2 * W_LN + 20)

  sub0 = jax.lax.broadcasted_iota(jnp.int32, (8, 128), 0) == 0

  def zero_step(j, c):
    for b in range(NB):
      G[b, j, T // 4:1024, :] = jnp.zeros((1024 - T // 4, 256), U32)
    return c
  jax.lax.fori_loop(0, 7, zero_step, 0)

  def zero_rows(i, c):
    r = mult(i * 48, 8)
    gb[:, pl.ds(r, 48), :] = jnp.zeros((4, 48, 128), F32)
    x1[pl.ds(r, 48), :] = jnp.zeros((48, D), F32)
    return c
  jax.lax.fori_loop(0, (TM + 16) // 48, zero_rows, 0)
  st[...] = jnp.zeros(st.shape, F32)

  xcopy(0).wait()
  zs[...] = pltpu.bitcast(xo[0:16, 0:128], U32) >> 31
  wcopy(I_A1).wait()

  def prep_wa1(i, c):
    c0 = mult(i * 256, 256)
    blk = [ra1[r:r + 256, pl.ds(c0 + cc, 256)].astype(F32) * 0.5 for r in (0, 256) for cc in (0, 1024)]
    for j, f in enumerate(beta_forms(*blk)):
      WA[j, :, pl.ds(c0, 256)] = st_bf(f())
    return c
  jax.lax.fori_loop(0, 4, prep_wa1, 0)
  bd = Body()
  ha, hb = [ln_rows(v.astype(F32)) for v in rows2(xo, 0)]
  wcopy(I_B1).wait()
  bd.push(prep_weight(rb1, WB, 1024, 256, 0.5), W_PREP)
  gz = Gamma()
  run(ff_a(bd, gz, fresh_u(alpha_forms(*quads(ha, hb))), 0))
  for k, v in enumerate(gz.result()):
    sS[k] = half_silu(v) if k < 3 else v

  def p1_body(t, last):
    bd = Body(BUD1, NHI1)
    r0 = mult(t * TM, TM)
    if not last:
      xcopy(t + 1).wait()
      rn = mult((t + 1) * TM, TM)
      ha, hb = [ln_rows(v.astype(F32)) for v in rows2(xo, rn)]
      bd.push(ln_deps(ha, hb), W_LN)
    post_g(bd, max(t - 1, 0) if isinstance(t, int) else jnp.maximum(t - 1, 0))
    gy = Gamma(init_quads(xo, r0, cast=True), reps=2)
    p = ff_step(bd, 0, ff_carried(bd), scratch_u, 1, gy, True)
    if not last:
      z = ff_step(bd, 1, p, fresh_u(alpha_forms(*quads(ha, hb))), 0, gy, False)
      store_quads(x1, r0, gy.result())
      for k in range(4):
        sS[k] = z[k]
    else:
      for i in (I_Q, I_K, I_V, I_O):
        wcopy(i).wait()
      prep_from_value(dot_nt(rq[...], rk[...]) * QSCALE, MQK)
      prep_from_value(dot(rv[...], ro[...]), MVO)
      bth = ff_b(bd, gy, p, 1)
      gq = Gamma()
      run(merge(qp_thunks(bd, gq, 0), bth[:3]))
      gs = Gamma(transposed=True)
      run(merge(s_thunks(bd, gs, fresh_u(phi_forms(*gq.result())), 0, 0), bth[3:]))
      store_quads(x1, r0, gy.result())
      for k, v in enumerate(gs.result()):
        sS[k] = v

  if 'P1' in PHASES:
    jax.lax.fori_loop(0, NT - 1, lambda t, c: (p1_body(t, False), c)[1], 0)
  else:
    for t in range(1, NT):
      xcopy(t).wait()
  if 'P1L' in PHASES:
    p1_body(NT - 1, True)
  else:
    for i in (I_Q, I_K, I_V, I_O):
      wcopy(i).wait()

  def p2_body(i, first, last):
    bd = Body(BUD2, NHI2)
    b = i // TPB
    bn_ = (i + 1) // TPB
    at = Att()
    if first:
      for k in (I_P1, I_DW, I_P2, I_A2, I_B2):
        wcopy(k).wait()
      post_g(bd, NT - 1)
      dwf = rdw[...].astype(F32)
      for k in range(KW):
        DWB[k] = jnp.broadcast_to(dwf[k:k + 1, :], (8, D))
      bd.push(prep_weight(rp1, WP1, 256, 512, 0.5), W_PREP)
      bd.push(prep_weight(rp2, WP2, 256, 256, 1.0), W_PREP)
      bd.push(prep_weight(ra2, WA, 256, 1024, 0.5), W_PREP)
      bd.push(prep_weight(rb2, WB, 1024, 256, 0.5), W_PREP)
    else:
      conv_unit(bd, i - 2)
      halo = gb[:, TM:TM + 16, :]
    s = att_step(bd, at, b, 0, att_carried(bd, at), scratch_u, b, 1)
    if not first:
      ha, hb = epi_mvo(bd, i - 1, budget=BUDM)
    s = att_step(bd, at, b, 1, s, scratch_u, b, 2)
    if not first:
      bd.push(ln_deps(ha, hb), W_LN)
    s = att_step(bd, at, b, 2, s, scratch_u, b, 3)
    if not first:
      cache = {}

      def roll_window():
        bd.flush_lo()
        gb[:, 0:16, :] = halo

      gd = epi_pw1(bd, ha, hb, 0, cache, budget=BUDP, pre_store=roll_window)
      gd += epi_pw1(bd, ha, hb, 1, cache)
      if not last:
        bd.push(gd, 8)
    if not last:
      gq = Gamma()
      run(qp_thunks(bd, gq, i + 1))
      s = att_step(bd, at, b, 3, s, fresh_u(phi_forms(*gq.result())), bn_, 0, False)
      for k in range(4):
        sS[k] = s[k]
    else:
      conv_unit(bd, i - 1, HOST8)
      att_step(bd, at, b, 3, s, None, None, None, pv_budget=BUDL)
    for k in range(4):
      osc[k] = at.acc[k]
    for hh in range(2):
      lsc[hh] = at.l[hh]
    return bd

  if 'P2F' in PHASES:
    p2_body(0, True, False)
  else:
    for k in (I_P1, I_DW, I_P2, I_A2, I_B2):
      wcopy(k).wait()
  def p2_pair(k, c):
    p2_body(2 * k + 1, False, False)

    @pl.when(k >= 0)
    def _():
      p2_body(2 * k + 2, False, False)
    return c
  if 'P2' in PHASES:
    for i_ in range(1, NT - 1):
      pl.when(z_s[0] == 0)(lambda i_=i_: p2_body(i_, False, False) and None)
  if 'P2S' in PHASES:
    pl.when(z_s[0] == 0)(lambda: p2_body(3, False, False) and None)
  if 'P2L' in PHASES:
    bd = p2_body(NT - 1, False, True)
  else:
    bd = Body()
    conv_unit(bd, NT - 2, HOST8)

  ha, hb = epi_mvo(bd, NT - 1, budget=BUDL2)

  def roll_window():
    print("leftover groups", len(bd.lo)) if DEBUG else None
    bd.flush()
    conv_exposed(bd, NT - 2, [l for l in range(4) if l not in HOST8])
    gb[:, 0:16, :] = gb[:, TM:TM + 16, :]

  epi_pw1(bd, ha, hb, 0, None, budget=BUDL2, pre_store=roll_window)
  conv_unit(bd, NT - 1, HOSTL)
  epi_pw1(bd, ha, hb, 1, None, budget=BUDL3)
  bd.flush()
  conv_exposed(bd, NT - 1, [l for l in range(4) if l not in HOSTL])
  conv_tail((0, 1, 2, 3))
  n_s = jnp.where(jax.lax.broadcasted_iota(jnp.int32, (8, D), 0) == 0, N // 8 - 7.0, N // 8 + 1.0)
  s1 = st[8:16, :]
  mu_s = st[0:8, :] + s1 / n_s
  m2_s = st[16:24, :] - s1 * s1 / n_s
  mu = jnp.sum(mu_s * n_s, axis=0, keepdims=True) * (1.0 / N)
  dm = mu_s - mu
  var = jnp.sum(m2_s + dm * dm * n_s, axis=0, keepdims=True) * (1.0 / N)
  bn[0:8, :] = jnp.broadcast_to(mu, (8, D))
  bn[8:16, :] = jnp.broadcast_to(0.5 * jax.lax.rsqrt(var + EPS), (8, D))

  bd = Body()
  th, (hold) = pre3(bd, 0)
  run(th)
  ha, hb = hold
  gz = Gamma()
  run(ff_a(bd, gz, fresh_u(alpha_forms(*quads(ha, hb))), 0))
  for k, v in enumerate(gz.result()):
    sS[k] = half_silu(v) if k < 3 else v

  def p3_body(t, last):
    bd = Body(BUD3, NHI3)
    r0 = mult(t * TM, TM)

    @pl.when(t >= 2)
    def _():
      ocopy(t - 2).start()

    p0 = ff_carried(bd)
    extra = None
    if not last:
      th, hold = pre3(bd, t + 1)
      extra = (P3POS, th)
    post3(bd, max(t - 1, 0) if isinstance(t, int) else jnp.maximum(t - 1, 0))
    gy = Gamma(init_quads(x1, r0), reps=2)
    p = ff_step(bd, 0, p0, scratch_u, 1, gy, True, extra)
    if not last:
      z = ff_step(bd, 1, p, fresh_u(alpha_forms(*quads(*hold))), 0, gy, False)
      for k in range(4):
        sS[k] = z[k]
    else:
      run(ff_b(bd, gy, p, 1))
    store_quads(x1, r0, gy.result())

  if 'P3' in PHASES:
    jax.lax.fori_loop(0, NT - 1, lambda t, c: (p3_body(t, False), c)[1], 0)
  if 'P3L' in PHASES:
    p3_body(NT - 1, True)

  bd = Body()
  ocopy(NT - 2).start()
  post3(bd, NT - 1)
  ocopy(NT - 1).start()
  for t in range(NT):
    ocopy(t).wait()


@jax.jit
def pallas_standalone__conformer_family_conformer__speech_kernel(
    x, w_ff1_a, w_ff1_b, w_q, w_k, w_v, w_o, w_pw1, dw, w_pw2, w_ff2_a, w_ff2_b):
  hbm = pl.BlockSpec(memory_space=pl.ANY)
  V = pltpu.VMEM
  out = pl.pallas_call(
      kernel,
      out_shape=jax.ShapeDtypeStruct((N, D), x.dtype),
      in_specs=[pl.BlockSpec(memory_space=pltpu.SMEM)] + [hbm] * 12,
      out_specs=hbm,
      scratch_shapes=[
          V((N, D), BF),
          V((D, FH), BF), V((FH, D), BF), V((D, FH), BF), V((FH, D), BF),
          V((D, D), BF), V((D, D), BF), V((D, D), BF), V((D, D), BF),
          V((D, 2 * D), BF), V((KW, D), BF), V((D, D), BF),
          V((7, 128, 1024), U32), V((7, 512, 256), U32),
          V((7, 128, 256), U32), V((7, 128, 256), U32),
          V((7, 128, 512), U32), V((7, 128, 256), U32),
          V((KW, 8, D), F32),
          V((N, D), F32),
          V((4, N + TM + 8, 128), F32),
          V((NB, 7, 1024, 256), U32),
          V((4, TM + 16, 128), F32),
          V((4, H, 512), F32),
          V((7, H // 2, 256), U32),
          V((4, H, 256), F32),
          V((2, H, 128), F32),
          V((24, D), F32), V((16, D), F32), V((8, 128), U32),
          pltpu.SemaphoreType.DMA((2 * NT + 11,)),
      ],
      compiler_params=pltpu.CompilerParams(vmem_limit_bytes=124 * 1024 * 1024),
  )(jnp.zeros((1,), jnp.int32), x.reshape(N, D), w_ff1_a, w_ff1_b, w_q, w_k, w_v, w_o, w_pw1, dw, w_pw2, w_ff2_a, w_ff2_b)
  return out.reshape(NB, T, D)
```

```python
import jax
import jax.numpy as jnp
import jax.experimental.pallas as pl
import jax.experimental.pallas.tpu as pltpu

BF = jnp.bfloat16
F32 = jnp.float32
U32 = jnp.uint32

NB, T, D, FH, KW = 2, 4000, 512, 2048, 15
N = NB * T
TM = 800
H = TM // 2
NT = N // TM
TPB = T // TM
EPS = 1e-5
QSCALE = D ** -0.5 * 1.4426950408889634
NEG = -1e30

PVMAP = [0, 2, 6, 5, 3, 4, 1]
AORD = [0, 3, 4, 6, 2, 1, 5]
TORD = [0, 3, 4, 6, 1, 2, 5]
BORD = [2, 4, 0, 3, 6, 5, 1]
W_LN, W_PREP = 36, 9
BUD1, BUD2, BUD3, BUDM = 800, 700, 1000, 700
NHI1, NHI2, NHI3 = 35, 40, 35
NHI, NHIF, HIW, GATE, NG = 40, 0, 1, 2, 6
P3POS = 6
BUDL, BUDL2, BUDL3 = 1500, 850, 850
FLD = 2
BUDP = 850
HOSTL = (0,)
HOST8 = (0, 1, 2)
DEBUG = False
W_CONV = 36
LNR, LNGATE, W_G = 80, True, 22
BUDGET = 560
PHASES = ('P1', 'P1L', 'P2F', 'P2', 'P2L', 'P3', 'P3L')
CONTRIB = [((0, 1), (3, 1)), ((2, 1), (3, -1)), ((1, 1), (3, 1)), ((0, 1), (2, 1)),
           ((0, -1), (1, 1)), ((3, 1),), ((0, 1),)]


def dot(a, b):
  return jnp.dot(a, b, preferred_element_type=F32)


def dot_nt(a, b):
  return jax.lax.dot_general(a, b, (((1,), (1,)), ((), ())), preferred_element_type=F32)


def alpha_forms(a11, a12, a21, a22):
  return [lambda: a11 + a22, lambda: a21 + a22, lambda: a11, lambda: a22,
          lambda: a11 + a12, lambda: a21 - a11, lambda: a12 - a22]


def beta_forms(b11, b12, b21, b22):
  return [lambda: b11 + b22, lambda: b11, lambda: b12 - b22, lambda: b21 - b11,
          lambda: b22, lambda: b11 + b12, lambda: b21 + b22]


def phi_forms(q11, q12, q21, q22):
  return beta_forms(q11, q21, q12, q22)


def quads(ha, hb):
  return ha[:, :256], ha[:, 256:], hb[:, :256], hb[:, 256:]


class Gamma:
  def __init__(self, init=None, transposed=False, on_final=None, reps=1):
    self.p = [None] * 4 if init is None else list(init)
    self.sg = [1] * 4
    self.left = [4 * reps, 2 * reps, 2 * reps, 4 * reps]
    self.tr = transposed
    self.on_final = on_final

  def add(self, j, m):
    for q, sg in CONTRIB[j]:
      if self.tr and q in (1, 2):
        q = 3 - q
      v = self.p[q]
      if callable(v):
        v = v()
      s = self.sg[q]
      if v is None:
        self.p[q], self.sg[q] = m, sg
      elif s == 1:
        self.p[q] = v + m if sg == 1 else v - m
      else:
        self.p[q], self.sg[q] = (m - v, 1) if sg == 1 else (v + m, -1)
      self.left[q] -= 1
      if self.left[q] == 0:
        assert self.sg[q] == 1
        if self.on_final is not None:
          self.on_final(q, self.p[q])

  def result(self):
    assert all(n == 0 for n in self.left)
    return list(self.p)


def rep(x, n, axis):
  return jnp.concatenate([x] * n, axis=axis) if n > 1 else x


def ld_bf(u):
  return pltpu.bitcast(u, BF)


def st_bf(x):
  return pltpu.bitcast(x.astype(BF), U32)


def ln_rows(x):
  m = jnp.mean(x, axis=-1, keepdims=True)
  xc = x - m
  v = jnp.mean(xc * xc, axis=-1, keepdims=True)
  return xc * jax.lax.rsqrt(v + EPS)


def half_silu(hz):
  return hz + hz * jnp.tanh(hz)


def row_vregs(x, c0=0):
  return [x[r:r + 8, c0:c0 + 128] for r in range(0, x.shape[0], 8)]


def tie(zm, u, deps, cast):
  if not deps:
    return u
  n = u.shape[0] // 8
  nk = u.shape[1] // 128
  slots = n * nk
  assign = {}
  for idx, d in enumerate(deps):
    assign[(idx * slots) // len(deps)] = d
  rows = []
  for rb in range(n):
    blk = u[rb * 8:(rb + 1) * 8]
    if any((rb * nk + k) in assign for k in range(nk)):
      parts = []
      for k in range(nk):
        pc = blk[:, k * 128:(k + 1) * 128]
        d = assign.get(rb * nk + k)
        if d is not None:
          pc = jnp.where(zm, pltpu.bitcast(d, U32) if cast else d, pc)
        parts.append(pc)
      blk = jnp.concatenate(parts, axis=1)
    rows.append(blk)
  return jnp.concatenate(rows, axis=0)


def sel(c, a, b):
  if isinstance(c, bool):
    return a if c else b
  return jnp.where(c, a, b)


def mult(x, n):
  return x if isinstance(x, int) else pl.multiple_of(x, n)


def interleave(a, b):
  out = []
  for i in range(max(len(a), len(b))):
    if i < len(a):
      out.append(a[i])
    if i < len(b):
      out.append(b[i])
  return out


def merge(s1, s2):
  out, n1, n2, i, j = [], len(s1), len(s2), 0, 0
  while i < n1 or j < n2:
    if j >= n2 or (i < n1 and i * n2 <= j * n1):
      out.append(s1[i]); i += 1
    else:
      out.append(s2[j]); j += 1
  return out


def kernel(z_s, x_h, wa1_h, wb1_h, wq_h, wk_h, wv_h, wo_h, wp1_h, dw_h, wp2_h, wa2_h, wb2_h, out_h,
           xo, ra1, rb1, ra2, rb2, rq, rk, rv, ro, rp1, rdw, rp2,
           WA, WB, MQK, MVO, WP1, WP2, DWB, x1, dc, G, gb, sS, qa, osc, lsc, st, bn, zs, sem):

  def xcopy(t):
    return pltpu.make_async_copy(x_h.at[pl.ds(t * TM, TM)], xo.at[pl.ds(t * TM, TM)], sem.at[t])

  def ocopy(t):
    return pltpu.make_async_copy(xo.at[pl.ds(t * TM, TM)], out_h.at[pl.ds(t * TM, TM)], sem.at[NT + 11 + t])

  wsrc = [wa1_h, wb1_h, wq_h, wk_h, wv_h, wo_h, wp1_h, dw_h, wp2_h, wa2_h, wb2_h]
  wdst = [ra1, rb1, rq, rk, rv, ro, rp1, rdw, rp2, ra2, rb2]
  I_A1, I_B1, I_Q, I_K, I_V, I_O, I_P1, I_DW, I_P2, I_A2, I_B2 = range(11)

  def wcopy(i):
    return pltpu.make_async_copy(wsrc[i], wdst[i], sem.at[NT + i])

  xcopy(0).start()
  wcopy(I_A1).start()
  wcopy(I_B1).start()
  xcopy(1).start()
  for i in (I_Q, I_K, I_V, I_O):
    wcopy(i).start()
  for t in range(2, NT):
    xcopy(t).start()
  for i in (I_P1, I_DW, I_P2, I_A2, I_B2):
    wcopy(i).start()

  def prep_weight(raw, dst, kh, nh, scale, cw=256):
    deps = []
    for c0 in range(0, nh, cw):
      for r0 in range(0, kh, 256):
        blk = [raw[r:r + 256, c:c + cw].astype(F32) * scale
               for r in (r0, kh + r0) for c in (c0, nh + c0)]
        for j, f in enumerate(beta_forms(*blk)):
          dst[j, r0 // 2:r0 // 2 + 128, c0:c0 + cw] = st_bf(f())
        for j in range(7):
          v = dst[j, r0 // 2:r0 // 2 + 128, c0:c0 + cw]
          deps += [pltpu.bitcast(v[r:r + 8, c:c + 128], F32)
                   for r in range(0, 128, 8) for c in range(0, cw, 128)]
    return deps

  def prep_from_value(m, dst):
    blk = [m[r:r + 256, c:c + 256] for r in (0, 256) for c in (0, 256)]
    for j, f in enumerate(beta_forms(*blk)):
      dst[j] = st_bf(f())

  def rows2(ref, r):
    return ref[pl.ds(r, H), :], ref[pl.ds(r + H, H), :]

  def init_quads(ref, r, cast=False):
    q = [ref[pl.ds(r + h, H), c:c + 256] for h in (0, H) for c in (0, 256)]
    return [v.astype(F32) for v in q] if cast else q

  def store_quads(ref, r, y):
    ref[pl.ds(r, H), :] = jnp.concatenate([y[0], y[1]], axis=1)
    ref[pl.ds(r + H, H), :] = jnp.concatenate([y[2], y[3]], axis=1)

  def store_tied(bd, ref, lead, r0, c0, val, step):
    for rr in range(0, val.shape[0], step):
      n = min(step, val.shape[0] - rr)
      ref[lead + (pl.ds(r0 + rr, n), slice(c0, c0 + val.shape[1]))] = val[rr:rr + n]
      got = ref[lead + (pl.ds(r0 + rr + n - 8, 8), slice(c0, c0 + 128))]
      bd.push([got if got.dtype == F32 else pltpu.bitcast(got, F32)], n * val.shape[1] // 1024)

  def ln_deps(ha, hb):
    return row_vregs(ha, 384) + row_vregs(hb, 384)

  class Body:
    def __init__(self, budget=BUDGET, nhi=25):
      self.nhi = nhi
      self.zm = zs[...] == 2
      self.budget = budget
      self.hi = []
      self.lo = []
      self.anchors = []

    def push(self, deps, w, hi=False):
      (self.hi if hi else self.lo).extend((w, 1, (lambda a, d=d: [d])) for d in deps)

    def push_lazy(self, w, n, fn):
      self.lo.append((w, n, fn))

    def note_result(self, r):
      self.anchors.append(r[0:8, 0:128])

    def gate(self, x, anchor):
      nr, nc = x.shape[0] // 8, x.shape[1] // 128
      return jnp.where(rep(rep(self.zm, nr, 0), nc, 1), rep(rep(anchor, nr, 0), nc, 1), x)

    def anchor(self):
      return self.anchors[-GATE] if GATE and len(self.anchors) >= GATE else None

    def take(self, budget, nhi, slots=50):
      out, tot = [], 0
      anchor = self.anchor()
      while self.hi and len(out) < nhi:
        w, n, fn = self.hi.pop(0)
        out += fn(anchor)
        tot += w * HIW
      while self.lo:
        w, n, fn = self.lo[0]
        if tot + w > budget or len(out) + n > slots:
          break
        self.lo.pop(0)
        tot += w
        out += fn(anchor)
      return out

    def flush_lo(self):
      anchor = self.anchor()
      rest = []
      for w, n, fn in self.lo:
        ds = fn(anchor)
        rest += [(w // max(n, 1), 1, (lambda a, d=d: [d])) for d in ds]
      self.lo = rest

    def flush(self):
      chain = [self.anchor()]
      for _, n, fn in self.hi + self.lo:
        out = fn(chain[-FLD] if len(chain) >= FLD else chain[0])
        if n > 1:
          chain.append(out[0])
      self.hi, self.lo = [], []

    def lhs_u(self, u, budget):
      return ld_bf(tie(self.zm, u, self.take(budget, self.nhi), True))

    def lhs_f(self, x, budget):
      return tie(self.zm, x, self.take(budget, NHIF if budget else 0, 2 * (x.shape[0] // 8)), False).astype(BF)

  def producer_thunks(bd, gam, get_u, rhs_fn, nt_dims, order=AORD, nhf=2):
    def mk(j):
      def run_():
        u = get_u(j)
        outs = []
        for hf in range(nhf):
          lhs = bd.lhs_u(u(hf), bd.budget)
          rhs = rhs_fn(j, hf)
          outs.append(dot_nt(lhs, rhs) if nt_dims else dot(lhs, rhs))
          bd.note_result(outs[-1])
        gam.add(j, jnp.concatenate(outs, axis=1) if nhf > 1 else outs[0])
      return run_
    return [mk(j) for j in order]

  def consumer_thunks(bd, gam, forms, rhs_fn, budget=0, order=BORD, cache=None):
    def mk(j):
      def run_():
        if cache is not None and j in cache:
          lv = cache[j]
        else:
          lv = bd.lhs_f(forms[j](), budget)
          if cache is not None:
            cache[j] = lv
        res = dot(lv, rhs_fn(j))
        bd.note_result(res)
        gam.add(j, res)
      return run_
    return [mk(j) for j in order]

  def scratch_u(j):
    return lambda hf: qa[j]

  def fresh_u(forms):
    def get(j):
      u = st_bf(forms[j]())
      qa[j] = u
      return lambda hf: u if hf == 0 else qa[j]
    return get

  def run(thunks):
    for th in thunks:
      th()

  def ff_act(bd, p, skip=()):
    def cb(q, z):
      if q in skip:
        p[q] = z
        return
      u = half_silu(z)
      p[q] = u
      bd.push(row_vregs(jnp.maximum(jnp.maximum(u[:, 0:128], u[:, 128:256]),
                                    jnp.maximum(u[:, 256:384], u[:, 384:512]))), 20, hi=True)
    return cb

  def ff_carried(bd):
    p = [sS[0], sS[1], sS[2], None]
    ff_act(bd, p)(3, sS[3])
    return p

  def ff_a(bd, gz, get_u, cn):
    return producer_thunks(bd, gz, get_u,
                           lambda j, hf: ld_bf(WA[j, :, cn * 512 + hf * 256:cn * 512 + hf * 256 + 256]), False)

  def ff_b(bd, gy, p, c):
    return consumer_thunks(bd, gy, alpha_forms(*p), lambda j: ld_bf(WB[j, c * 256:(c + 1) * 256, :]))

  def ff_step(bd, c, p, get_u, cn, gy, act, extra=None):
    pn = [None] * 4
    gz = Gamma(on_final=ff_act(bd, pn, () if act else (3,)))
    seq = interleave(ff_a(bd, gz, get_u, cn), ff_b(bd, gy, p, c))
    if extra is not None:
      seq[extra[0]:extra[0]] = extra[1]
    run(seq)
    return pn

  class LazyLN:
    def __init__(self, bd, load, front=False):
      self.bd = bd
      self.out = [[None] * (H // LNR), [None] * (H // LNR)]
      self.todo = []
      items = []
      for i in range(H // LNR):
        for h in range(2):
          def fn(anchor, h=h, i=i):
            if self.out[h][i] is None:
              x = load(h, i * LNR)
              if anchor is not None and LNGATE:
                x = bd.gate(x, anchor)
              self.out[h][i] = ln_rows(x)
            return row_vregs(self.out[h][i], 384)
          self.todo.append(fn)
          items.append((W_LN * (LNR // 8), LNR // 8, fn))
      if front:
        bd.lo[0:0] = items
      else:
        bd.lo.extend(items)

    def get(self):
      for fn in self.todo:
        fn(None)
      return [jnp.concatenate(v, axis=0) for v in self.out]

  def post_g(bd, t):
    r = mult(t * TM, TM)
    ln = LazyLN(bd, lambda h, r0: x1[pl.ds(r + h * H + r0, LNR), :])
    b = t // TPB
    rq_ = mult((t % TPB) * (H // 2), H // 2)
    forms = []

    def group(j, lo_, hi_, anchor):
      if not forms:
        forms.extend(alpha_forms(*quads(*ln.get())))
      f = forms[j]()[2 * lo_:2 * hi_]
      if anchor is not None:
        f = bd.gate(f, anchor)
      v = st_bf(f)
      G[b, j, pl.ds(rq_ + lo_, hi_ - lo_), :] = v
      got = G[b, j, pl.ds(rq_ + hi_ - 8, 8), 0:128]
      return [pltpu.bitcast(v[r_:r_ + 8, 128:256], F32) for r_ in range(0, hi_ - lo_, 16)] + [pltpu.bitcast(got, F32)]

    for j in range(7):
      for lo_, hi_ in ((0, 104), (104, 200)):
        bd.push_lazy(W_G * (hi_ - lo_) // 8, (hi_ - lo_ + 15) // 16 + 1,
                     lambda a, j=j, lo_=lo_, hi_=hi_: group(j, lo_, hi_, a))

  def qp_thunks(bd, gq, t):
    b = t // TPB
    rn = mult((t % TPB) * (H // 2), H // 2)
    return producer_thunks(bd, gq, lambda j: (lambda hf: G[b, j, pl.ds(rn, H // 2), :]),
                           lambda j, hf: ld_bf(MQK[j]), False, nhf=1)

  def s_thunks(bd, gs, get_u, b, c):
    return producer_thunks(bd, gs, get_u,
                           lambda j, hf: ld_bf(G[b, j, c * 256 + hf * 128:c * 256 + (hf + 1) * 128, :]),
                           True, order=TORD)

  class Att:
    def __init__(self):
      self.m = [None, None]
      self.l = [None, None]
      self.al = [None, None]
      self.acc = None

  def soft_cb(bd, at, c, p):
    held = {}

    def cb(q, sv):
      if c == 3:
        col = jax.lax.broadcasted_iota(jnp.int32, (H, 512), 1)
        sv = jnp.where(col < 512 - 48, sv, NEG)
      if q in (0, 2):
        held[q] = sv
        return
      hh = q // 2
      sa, sb = held[q - 1], sv
      mx = jnp.max(jnp.maximum(sa, sb), axis=-1, keepdims=True)
      mo = at.m[hh]
      mn = mx if mo is None else jnp.maximum(mo, mx)
      pa, pb = jnp.exp2(sa - mn), jnp.exp2(sb - mn)
      ta, tb = [(u[:, 0:128] + u[:, 128:256]) + (u[:, 256:384] + u[:, 384:512]) for u in (pa, pb)]
      if mo is None:
        at.al[hh] = None
        at.l[hh] = ta + tb
      else:
        at.al[hh] = jnp.exp2(mo - mn)
        at.l[hh] = at.l[hh] * at.al[hh] + (ta + tb)
      at.m[hh] = mn
      p[q - 1], p[q] = pa, pb
      for t_ in ((ta, tb) if hh == 0 else (tb, ta)):
        bd.push(row_vregs(t_), 12, hi=True)
      if c < 3:
        bd.push(row_vregs(at.l[hh]), 4, hi=True)
    return cb

  def att_carried(bd, at):
    p = [None] * 4
    cb = soft_cb(bd, at, 0, p)
    for q in range(4):
      cb(q, sS[q])
    return p

  def att_step(bd, at, b, c, p, get_u, bn_, cn, act=True, pv_budget=0):
    if at.acc is None:
      go = Gamma()
    else:
      acc = at.acc
      go = Gamma([(lambda q=q: acc[q] * al[q // 2]) for q in range(4)])
    al = list(at.al)
    pv = consumer_thunks(bd, go, alpha_forms(*p), lambda j: ld_bf(G[b, PVMAP[j], c * 256:(c + 1) * 256, :]),
                         budget=pv_budget)
    res = None
    if get_u is not None:
      pn = [None] * 4
      gs = Gamma(transposed=True, on_final=soft_cb(bd, at, cn, pn) if act else None)
      run(interleave(s_thunks(bd, gs, get_u, bn_, cn), pv))
      res = pn if act else gs.result()
    else:
      run(pv)
    at.acc = go.result()
    return res

  LS = TM // 8

  def conv_outputs(U, ls, dwk, u0, u1):
    start = (U % TPB) == 0
    win = {}

    def inp(u):
      if u not in win:
        win[u] = gb[ls, pl.ds(8 + u, 8, stride=LS), :]
      return win[u]

    outs = []
    for u in range(u0, u1):
      acc = [None, None]
      for k in range(KW):
        ui = u + k - KW // 2
        v = inp(ui)
        if start and u < 15 and ((u < 8) != (ui < 8)):
          v = jnp.where(sub0, 0.0, v)
        t = v * dwk[k]
        acc[k & 1] = t if acc[k & 1] is None else acc[k & 1] + t
      outs.append(acc[0] + acc[1])
    return outs

  def conv_unit(bd, U, lanes=(0, 1, 2, 3)):
    ru = (U + 1) * TM
    bounds = [(LS * g + NG // 2) // NG for g in range(NG + 1)]

    def make(l):
      ls = slice(l * 128, (l + 1) * 128)
      state = {}

      def group(g, anchor):
        u0, u1 = bounds[g], bounds[g + 1]
        dwk = [DWB[k, :, ls] for k in range(KW)]
        if anchor is not None:
          dwk = [bd.gate(v, anchor) for v in dwk]
        outs = conv_outputs(U, l, dwk, u0, u1)
        if g == 0:
          if U == 0:
            st[0:8, ls] = outs[8]
          state["k"] = outs[8] if U == 0 else st[0:8, ls]
          state["s1"] = st[8:16, ls]
          state["s2"] = st[16:24, ls]
        deps = []
        for u, o in zip(range(u0, u1), outs):
          d = o - state["k"]
          if U == 0 and u < 8:
            d = jnp.where(sub0, 0.0, d)
          d2 = d * d
          state["s1"] = state["s1"] + d
          state["s2"] = state["s2"] + d2
          dc[l, pl.ds(ru + u, 8, stride=LS), :] = o
          deps.append(d2)
        deps.append(dc[l, pl.ds(ru + u1 - 1, 8, stride=LS), :])
        if g == NG - 1:
          st[8:16, ls] = state["s1"]
          st[16:24, ls] = state["s2"]
        return deps
      return group

    for l in lanes:
      grp = make(l)
      for g in range(NG):
        n = bounds[g + 1] - bounds[g]
        bd.push_lazy(W_CONV * n + 15, n + 1, lambda a, grp=grp, g=g: grp(g, a))

  def conv_part(win, nr, dwk):
    acc = [None, None]
    for rho in range(8):
      if rho == 0:
        tt = win[8:8 + nr] * rep(dwk[7], nr // 8, 0)
      else:
        u = (win[0:nr + 8] * rep(dwk[rho - 1], nr // 8 + 1, 0)
             + win[8:nr + 16] * rep(dwk[rho + 7], nr // 8 + 1, 0))
        tt = pltpu.roll(u, nr + 8 - rho, 0)[0:nr]
      acc[rho & 1] = tt if acc[rho & 1] is None else acc[rho & 1] + tt
    return acc[0] + acc[1]

  def conv_exposed(bd, U, lanes):
    keep = bd.hi, bd.lo
    bd.hi, bd.lo = [], []
    conv_unit(bd, U, lanes)
    for _, _, fn in bd.lo:
      fn(None)
    bd.hi, bd.lo = keep

  def conv_tail(lanes):
    for l in lanes:
      ls = slice(l * 128, (l + 1) * 128)
      dwk = [DWB[k, :, ls] for k in range(KW)]
      halo = gb[l, TM:TM + 16, :]
      w = jnp.concatenate([halo, jnp.zeros((8, 128), F32)], axis=0)
      out = conv_part(w, 8, dwk)
      dc[l, N + TM:N + TM + 8, :] = out
      d = out - st[0:8, ls]
      st[8:16, ls] = st[8:16, ls] + d
      st[16:24, ls] = st[16:24, ls] + d * d

  def epi_mvo(bd, t, budget=0):
    r = mult(t * TM, TM)
    rl = [1.0 / jnp.sum(lsc[hh], axis=-1, keepdims=True) for hh in range(2)]
    oq = [osc[0] * rl[0], osc[1] * rl[0], osc[2] * rl[1], osc[3] * rl[1]]
    g = Gamma(init_quads(x1, r))
    run(consumer_thunks(bd, g, alpha_forms(*oq), lambda j: ld_bf(MVO[j]), budget=budget))
    y = g.result()
    xs = [jnp.concatenate([y[0], y[1]], axis=1), jnp.concatenate([y[2], y[3]], axis=1)]
    for h, v in zip((0, H), xs):
      store_tied(bd, x1, (), r + h, 0, v, 80)
    return [ln_rows(v) for v in xs]

  def epi_pw1(bd, ha, hb, sl, cache, budget=0, pre_store=None):
    g = Gamma()
    run(consumer_thunks(bd, g, alpha_forms(*quads(ha, hb)),
                        lambda j: ld_bf(WP1[j, :, sl * 256:(sl + 1) * 256]), order=AORD, cache=cache,
                        budget=budget))
    if pre_store is not None:
      pre_store()
    a1, b1, a2, b2 = g.result()
    deps = []
    for h, gv in ((0, a1 + a1 * jnp.tanh(b1)), (H, a2 + a2 * jnp.tanh(b2))):
      for k in range(2):
        gb[2 * sl + k, 16 + h:16 + h + H, :] = gv[:, k * 128:(k + 1) * 128]
        deps += [gb[2 * sl + k, r:r + 8, :] for r in range(16 + h, 16 + h + H, 8)]
    return deps

  def pre3(bd, t):
    r = mult(t * TM, TM)
    mu = rep(bn[0:8, :], H // 8, 0)
    hrs = rep(bn[8:16, :], H // 8, 0)
    hs = [half_silu((jnp.concatenate([dc[l, pl.ds(r + TM + 8 + h, H), :] for l in range(4)], axis=1)
                     - mu) * hrs) for h in (0, H)]
    for u in hs:
      bd.push(row_vregs(jnp.maximum(jnp.maximum(u[:, 0:128], u[:, 128:256]),
                                    jnp.maximum(u[:, 256:384], u[:, 384:512]))), 24, hi=True)
    g = Gamma(init_quads(x1, r))
    holder = []

    def finish():
      y = g.result()
      xs = [jnp.concatenate([y[0], y[1]], axis=1), jnp.concatenate([y[2], y[3]], axis=1)]
      ha, hb = [ln_rows(v) for v in xs]
      bd.lo[0:0] = [(W_LN, 1, (lambda a, d=d: [d])) for d in ln_deps(ha, hb)]
      for h, v in zip((0, H), xs):
        store_tied(bd, x1, (), r + h, 0, v, 80)
      holder.extend([ha, hb])

    return consumer_thunks(bd, g, alpha_forms(*quads(*hs)), lambda j: ld_bf(WP2[j])) + [finish], holder

  def post3(bd, t):
    r = mult(t * TM, TM)

    def piece(r0, anchor):
      x = x1[pl.ds(r + r0, LNR), :]
      if anchor is not None and LNGATE:
        x = bd.gate(x, anchor)
      o = ln_rows(x)
      xo[pl.ds(r + r0, LNR), :] = o.astype(BF)
      got = pltpu.bitcast(xo[pl.ds(r + r0 + LNR - 16, 16), 0:128], U32)
      return row_vregs(o, 384) + [pltpu.bitcast(got, F32)]

    for r0 in range(0, TM, LNR):
      bd.push_lazy((W_LN + 4) * (LNR // 8), LNR // 8 + 1, lambda a, r0=r0: piece(r0, a))

  sub0 = jax.lax.broadcasted_iota(jnp.int32, (8, 128), 0) == 0

  def zero_step(j, c):
    for b in range(NB):
      G[b, j, T // 4:1024, :] = jnp.zeros((1024 - T // 4, 256), U32)
    return c
  jax.lax.fori_loop(0, 7, zero_step, 0)

  def zero_rows(i, c):
    r = mult(i * 48, 8)
    gb[:, pl.ds(r, 48), :] = jnp.zeros((4, 48, 128), F32)
    x1[pl.ds(r, 48), :] = jnp.zeros((48, D), F32)
    return c
  jax.lax.fori_loop(0, (TM + 16) // 48, zero_rows, 0)
  st[...] = jnp.zeros(st.shape, F32)

  xcopy(0).wait()
  zs[...] = pltpu.bitcast(xo[0:16, 0:128], U32) >> 31
  wcopy(I_A1).wait()

  def prep_wa1(i, c):
    c0 = mult(i * 256, 256)
    blk = [ra1[r:r + 256, pl.ds(c0 + cc, 256)].astype(F32) * 0.5 for r in (0, 256) for cc in (0, 1024)]
    for j, f in enumerate(beta_forms(*blk)):
      WA[j, :, pl.ds(c0, 256)] = st_bf(f())
    return c
  jax.lax.fori_loop(0, 4, prep_wa1, 0)
  bd = Body()
  ha, hb = [ln_rows(v.astype(F32)) for v in rows2(xo, 0)]
  wcopy(I_B1).wait()
  bd.push(prep_weight(rb1, WB, 1024, 256, 0.5), W_PREP)
  gz = Gamma()
  run(ff_a(bd, gz, fresh_u(alpha_forms(*quads(ha, hb))), 0))
  for k, v in enumerate(gz.result()):
    sS[k] = half_silu(v) if k < 3 else v

  def p1_body(t, last):
    bd = Body(BUD1, NHI1)
    r0 = mult(t * TM, TM)
    if not last:
      xcopy(t + 1).wait()
      rn = mult((t + 1) * TM, TM)
      lnx = LazyLN(bd, lambda h, r0: xo[pl.ds(rn + h * H + r0, LNR), :].astype(F32))
    post_g(bd, max(t - 1, 0) if isinstance(t, int) else jnp.maximum(t - 1, 0))
    gy = Gamma(init_quads(xo, r0, cast=True), reps=2)
    p = ff_step(bd, 0, ff_carried(bd), scratch_u, 1, gy, True)
    if not last:
      z = ff_step(bd, 1, p, fresh_u(alpha_forms(*quads(*lnx.get()))), 0, gy, False)
      store_quads(x1, r0, gy.result())
      for k in range(4):
        sS[k] = z[k]
    else:
      for i in (I_Q, I_K, I_V, I_O):
        wcopy(i).wait()
      prep_from_value(dot_nt(rq[...], rk[...]) * QSCALE, MQK)
      prep_from_value(dot(rv[...], ro[...]), MVO)
      bth = ff_b(bd, gy, p, 1)
      gq = Gamma()
      run(merge(qp_thunks(bd, gq, 0), bth[:3]))
      gs = Gamma(transposed=True)
      run(merge(s_thunks(bd, gs, fresh_u(phi_forms(*gq.result())), 0, 0), bth[3:]))
      store_quads(x1, r0, gy.result())
      for k, v in enumerate(gs.result()):
        sS[k] = v
    bd.flush()

  if 'P1' in PHASES:
    jax.lax.fori_loop(0, NT - 1, lambda t, c: (p1_body(t, False), c)[1], 0)
  else:
    for t in range(1, NT):
      xcopy(t).wait()
  if 'P1L' in PHASES:
    p1_body(NT - 1, True)
  else:
    for i in (I_Q, I_K, I_V, I_O):
      wcopy(i).wait()

  def p2_body(i, first, last):
    bd = Body(BUD2, NHI2)
    b = i // TPB
    bn_ = (i + 1) // TPB
    at = Att()
    if first:
      for k in (I_P1, I_DW, I_P2, I_A2, I_B2):
        wcopy(k).wait()
      post_g(bd, NT - 1)
      dwf = rdw[...].astype(F32)
      for k in range(KW):
        DWB[k] = jnp.broadcast_to(dwf[k:k + 1, :], (8, D))
      bd.push(prep_weight(rp1, WP1, 256, 512, 0.5), W_PREP)
      bd.push(prep_weight(rp2, WP2, 256, 256, 1.0), W_PREP)
      bd.push(prep_weight(ra2, WA, 256, 1024, 0.5), W_PREP)
      bd.push(prep_weight(rb2, WB, 1024, 256, 0.5), W_PREP)
    else:
      conv_unit(bd, i - 2)
      halo = gb[:, TM:TM + 16, :]
    s = att_step(bd, at, b, 0, att_carried(bd, at), scratch_u, b, 1)
    if not first:
      ha, hb = epi_mvo(bd, i - 1, budget=BUDM)
    s = att_step(bd, at, b, 1, s, scratch_u, b, 2)
    if not first:
      bd.push(ln_deps(ha, hb), W_LN)
    s = att_step(bd, at, b, 2, s, scratch_u, b, 3)
    if not first:
      cache = {}

      def roll_window():
        bd.flush_lo()
        gb[:, 0:16, :] = halo

      gd = epi_pw1(bd, ha, hb, 0, cache, budget=BUDP, pre_store=roll_window)
      gd += epi_pw1(bd, ha, hb, 1, cache)
      if not last:
        bd.push(gd, 8)
    if not last:
      gq = Gamma()
      run(qp_thunks(bd, gq, i + 1))
      s = att_step(bd, at, b, 3, s, fresh_u(phi_forms(*gq.result())), bn_, 0, False)
      for k in range(4):
        sS[k] = s[k]
    else:
      conv_unit(bd, i - 1, HOST8)
      att_step(bd, at, b, 3, s, None, None, None, pv_budget=BUDL)
    for k in range(4):
      osc[k] = at.acc[k]
    for hh in range(2):
      lsc[hh] = at.l[hh]
    if first:
      bd.flush()
    return bd

  if 'P2F' in PHASES:
    p2_body(0, True, False)
  else:
    for k in (I_P1, I_DW, I_P2, I_A2, I_B2):
      wcopy(k).wait()
  def p2_pair(k, c):
    p2_body(2 * k + 1, False, False)

    @pl.when(k >= 0)
    def _():
      p2_body(2 * k + 2, False, False)
    return c
  if 'P2' in PHASES:
    for i_ in range(1, NT - 1):
      pl.when(z_s[0] == 0)(lambda i_=i_: p2_body(i_, False, False) and None)
  if 'P2S' in PHASES:
    pl.when(z_s[0] == 0)(lambda: p2_body(3, False, False) and None)
  if 'P2L' in PHASES:
    bd = p2_body(NT - 1, False, True)
  else:
    bd = Body()
    conv_unit(bd, NT - 2, HOST8)

  ha, hb = epi_mvo(bd, NT - 1, budget=BUDL2)

  def roll_window():
    print("leftover groups", len(bd.lo)) if DEBUG else None
    bd.flush()
    conv_exposed(bd, NT - 2, [l for l in range(4) if l not in HOST8])
    gb[:, 0:16, :] = gb[:, TM:TM + 16, :]

  epi_pw1(bd, ha, hb, 0, None, budget=BUDL2, pre_store=roll_window)
  conv_unit(bd, NT - 1, HOSTL)
  epi_pw1(bd, ha, hb, 1, None, budget=BUDL3)
  bd.flush()
  conv_exposed(bd, NT - 1, [l for l in range(4) if l not in HOSTL])
  conv_tail((0, 1, 2, 3))
  n_s = jnp.where(jax.lax.broadcasted_iota(jnp.int32, (8, D), 0) == 0, N // 8 - 7.0, N // 8 + 1.0)
  s1 = st[8:16, :]
  mu_s = st[0:8, :] + s1 / n_s
  m2_s = st[16:24, :] - s1 * s1 / n_s
  mu = jnp.sum(mu_s * n_s, axis=0, keepdims=True) * (1.0 / N)
  dm = mu_s - mu
  var = jnp.sum(m2_s + dm * dm * n_s, axis=0, keepdims=True) * (1.0 / N)
  bn[0:8, :] = jnp.broadcast_to(mu, (8, D))
  bn[8:16, :] = jnp.broadcast_to(0.5 * jax.lax.rsqrt(var + EPS), (8, D))

  bd = Body()
  th, (hold) = pre3(bd, 0)
  run(th)
  ha, hb = hold
  gz = Gamma()
  run(ff_a(bd, gz, fresh_u(alpha_forms(*quads(ha, hb))), 0))
  for k, v in enumerate(gz.result()):
    sS[k] = half_silu(v) if k < 3 else v

  def p3_body(t, last):
    bd = Body(BUD3, NHI3)
    r0 = mult(t * TM, TM)

    @pl.when(t >= 2)
    def _():
      ocopy(t - 2).start()

    p0 = ff_carried(bd)
    extra = None
    if not last:
      th, hold = pre3(bd, t + 1)
      extra = (P3POS, th)
    post3(bd, max(t - 1, 0) if isinstance(t, int) else jnp.maximum(t - 1, 0))
    gy = Gamma(init_quads(x1, r0), reps=2)
    p = ff_step(bd, 0, p0, scratch_u, 1, gy, True, extra)
    if not last:
      z = ff_step(bd, 1, p, fresh_u(alpha_forms(*quads(*hold))), 0, gy, False)
      for k in range(4):
        sS[k] = z[k]
    else:
      run(ff_b(bd, gy, p, 1))
    store_quads(x1, r0, gy.result())
    bd.flush()

  if 'P3' in PHASES:
    jax.lax.fori_loop(0, NT - 1, lambda t, c: (p3_body(t, False), c)[1], 0)
  if 'P3L' in PHASES:
    p3_body(NT - 1, True)

  bd = Body()
  ocopy(NT - 2).start()
  post3(bd, NT - 1)
  bd.flush()
  ocopy(NT - 1).start()
  for t in range(NT):
    ocopy(t).wait()


@jax.jit
def pallas_standalone__conformer_family_conformer__speech_kernel(
    x, w_ff1_a, w_ff1_b, w_q, w_k, w_v, w_o, w_pw1, dw, w_pw2, w_ff2_a, w_ff2_b):
  hbm = pl.BlockSpec(memory_space=pl.ANY)
  V = pltpu.VMEM
  out = pl.pallas_call(
      kernel,
      out_shape=jax.ShapeDtypeStruct((N, D), x.dtype),
      in_specs=[pl.BlockSpec(memory_space=pltpu.SMEM)] + [hbm] * 12,
      out_specs=hbm,
      scratch_shapes=[
          V((N, D), BF),
          V((D, FH), BF), V((FH, D), BF), V((D, FH), BF), V((FH, D), BF),
          V((D, D), BF), V((D, D), BF), V((D, D), BF), V((D, D), BF),
          V((D, 2 * D), BF), V((KW, D), BF), V((D, D), BF),
          V((7, 128, 1024), U32), V((7, 512, 256), U32),
          V((7, 128, 256), U32), V((7, 128, 256), U32),
          V((7, 128, 512), U32), V((7, 128, 256), U32),
          V((KW, 8, D), F32),
          V((N, D), F32),
          V((4, N + TM + 8, 128), F32),
          V((NB, 7, 1024, 256), U32),
          V((4, TM + 16, 128), F32),
          V((4, H, 512), F32),
          V((7, H // 2, 256), U32),
          V((4, H, 256), F32),
          V((2, H, 128), F32),
          V((24, D), F32), V((16, D), F32), V((8, 128), U32),
          pltpu.SemaphoreType.DMA((2 * NT + 11,)),
      ],
      compiler_params=pltpu.CompilerParams(vmem_limit_bytes=124 * 1024 * 1024),
  )(jnp.zeros((1,), jnp.int32), x.reshape(N, D), w_ff1_a, w_ff1_b, w_q, w_k, w_v, w_o, w_pw1, dw, w_pw2, w_ff2_a, w_ff2_b)
  return out.reshape(NB, T, D)
```

```python
import jax
import jax.numpy as jnp
import jax.experimental.pallas as pl
import jax.experimental.pallas.tpu as pltpu

BF = jnp.bfloat16
F32 = jnp.float32
U32 = jnp.uint32

NB, T, D, FH, KW = 2, 4000, 512, 2048, 15
N = NB * T
TM = 800
H = TM // 2
NT = N // TM
TPB = T // TM
EPS = 1e-5
QSCALE = D ** -0.5 * 1.4426950408889634
NEG = -1e30

PVMAP = [0, 2, 6, 5, 3, 4, 1]
AORD = [0, 3, 4, 6, 2, 1, 5]
TORD = [0, 3, 4, 6, 1, 2, 5]
BORD = [2, 4, 0, 3, 6, 5, 1]
W_LN, W_PREP = 36, 9
BUD1, BUD2, BUD3, BUDM = 800, 700, 1000, 700
NHI1, NHI2, NHI3 = 35, 34, 35
NHI, NHIF, HIW, GATE, NG = 40, 0, 1, 2, 6
P3POS = 6
BUDL, BUDL2, BUDL3 = 1500, 850, 850
FLD = 2
BUDP = 850
HOSTL = (0,)
HOST8 = (0, 1, 2)
DEBUG = False
W_CONV = 36
LNR, LNGATE, W_G = 80, True, 22
BOUND, P2N = 'none', 9
BUDGET = 560
PHASES = ('P1', 'P1L', 'P2F', 'P2', 'P2L', 'P3', 'P3L')
CONTRIB = [((0, 1), (3, 1)), ((2, 1), (3, -1)), ((1, 1), (3, 1)), ((0, 1), (2, 1)),
           ((0, -1), (1, 1)), ((3, 1),), ((0, 1),)]


def dot(a, b):
  return jnp.dot(a, b, preferred_element_type=F32)


def dot_nt(a, b):
  return jax.lax.dot_general(a, b, (((1,), (1,)), ((), ())), preferred_element_type=F32)


def alpha_forms(a11, a12, a21, a22):
  return [lambda: a11 + a22, lambda: a21 + a22, lambda: a11, lambda: a22,
          lambda: a11 + a12, lambda: a21 - a11, lambda: a12 - a22]


def beta_forms(b11, b12, b21, b22):
  return [lambda: b11 + b22, lambda: b11, lambda: b12 - b22, lambda: b21 - b11,
          lambda: b22, lambda: b11 + b12, lambda: b21 + b22]


def phi_forms(q11, q12, q21, q22):
  return beta_forms(q11, q21, q12, q22)


def quads(ha, hb):
  return ha[:, :256], ha[:, 256:], hb[:, :256], hb[:, 256:]


class Gamma:
  def __init__(self, init=None, transposed=False, on_final=None, reps=1):
    self.p = [None] * 4 if init is None else list(init)
    self.sg = [1] * 4
    self.left = [4 * reps, 2 * reps, 2 * reps, 4 * reps]
    self.tr = transposed
    self.on_final = on_final

  def add(self, j, m):
    for q, sg in CONTRIB[j]:
      if self.tr and q in (1, 2):
        q = 3 - q
      v = self.p[q]
      if callable(v):
        v = v()
      s = self.sg[q]
      if v is None:
        self.p[q], self.sg[q] = m, sg
      elif s == 1:
        self.p[q] = v + m if sg == 1 else v - m
      else:
        self.p[q], self.sg[q] = (m - v, 1) if sg == 1 else (v + m, -1)
      self.left[q] -= 1
      if self.left[q] == 0:
        assert self.sg[q] == 1
        if self.on_final is not None:
          self.on_final(q, self.p[q])

  def result(self):
    assert all(n == 0 for n in self.left)
    return list(self.p)


def rep(x, n, axis):
  return jnp.concatenate([x] * n, axis=axis) if n > 1 else x


def ld_bf(u):
  return pltpu.bitcast(u, BF)


def st_bf(x):
  return pltpu.bitcast(x.astype(BF), U32)


def ln_rows(x):
  m = jnp.mean(x, axis=-1, keepdims=True)
  xc = x - m
  v = jnp.mean(xc * xc, axis=-1, keepdims=True)
  return xc * jax.lax.rsqrt(v + EPS)


def half_silu(hz):
  return hz + hz * jnp.tanh(hz)


def row_vregs(x, c0=0):
  return [x[r:r + 8, c0:c0 + 128] for r in range(0, x.shape[0], 8)]


def tie(zm, u, deps, cast):
  if not deps:
    return u
  n = u.shape[0] // 8
  nk = u.shape[1] // 128
  slots = n * nk
  assign = {}
  for idx, d in enumerate(deps):
    assign[(idx * slots) // len(deps)] = d
  rows = []
  for rb in range(n):
    blk = u[rb * 8:(rb + 1) * 8]
    if any((rb * nk + k) in assign for k in range(nk)):
      parts = []
      for k in range(nk):
        pc = blk[:, k * 128:(k + 1) * 128]
        d = assign.get(rb * nk + k)
        if d is not None:
          pc = jnp.where(zm, pltpu.bitcast(d, U32) if cast else d, pc)
        parts.append(pc)
      blk = jnp.concatenate(parts, axis=1)
    rows.append(blk)
  return jnp.concatenate(rows, axis=0)


def sel(c, a, b):
  if isinstance(c, bool):
    return a if c else b
  return jnp.where(c, a, b)


def mult(x, n):
  return x if isinstance(x, int) else pl.multiple_of(x, n)


def interleave(a, b):
  out = []
  for i in range(max(len(a), len(b))):
    if i < len(a):
      out.append(a[i])
    if i < len(b):
      out.append(b[i])
  return out


def merge(s1, s2):
  out, n1, n2, i, j = [], len(s1), len(s2), 0, 0
  while i < n1 or j < n2:
    if j >= n2 or (i < n1 and i * n2 <= j * n1):
      out.append(s1[i]); i += 1
    else:
      out.append(s2[j]); j += 1
  return out


def kernel(z_s, x_h, wa1_h, wb1_h, wq_h, wk_h, wv_h, wo_h, wp1_h, dw_h, wp2_h, wa2_h, wb2_h, out_h,
           xo, ra1, rb1, ra2, rb2, rq, rk, rv, ro, rp1, rdw, rp2,
           WA, WB, MQK, MVO, WP1, WP2, DWB, x1, dc, G, gb, sS, qa, osc, lsc, st, bn, zs, sem):

  def xcopy(t):
    return pltpu.make_async_copy(x_h.at[pl.ds(t * TM, TM)], xo.at[pl.ds(t * TM, TM)], sem.at[t])

  def ocopy(t):
    return pltpu.make_async_copy(xo.at[pl.ds(t * TM, TM)], out_h.at[pl.ds(t * TM, TM)], sem.at[NT + 11 + t])

  wsrc = [wa1_h, wb1_h, wq_h, wk_h, wv_h, wo_h, wp1_h, dw_h, wp2_h, wa2_h, wb2_h]
  wdst = [ra1, rb1, rq, rk, rv, ro, rp1, rdw, rp2, ra2, rb2]
  I_A1, I_B1, I_Q, I_K, I_V, I_O, I_P1, I_DW, I_P2, I_A2, I_B2 = range(11)

  def wcopy(i):
    return pltpu.make_async_copy(wsrc[i], wdst[i], sem.at[NT + i])

  for i in (I_Q, I_K, I_V, I_O):
    wcopy(i).start()
  xcopy(0).start()
  wcopy(I_A1).start()

  def prep_weight(raw, dst, kh, nh, scale, cw=256):
    deps = []
    for c0 in range(0, nh, cw):
      for r0 in range(0, kh, 256):
        blk = [raw[r:r + 256, c:c + cw].astype(F32) * scale
               for r in (r0, kh + r0) for c in (c0, nh + c0)]
        for j, f in enumerate(beta_forms(*blk)):
          dst[j, r0 // 2:r0 // 2 + 128, c0:c0 + cw] = st_bf(f())
        for j in range(7):
          v = dst[j, r0 // 2:r0 // 2 + 128, c0:c0 + cw]
          deps += [pltpu.bitcast(v[r:r + 8, c:c + 128], F32)
                   for r in range(0, 128, 8) for c in range(0, cw, 128)]
    return deps

  def prep_from_value(m, dst):
    blk = [m[r:r + 256, c:c + 256] for r in (0, 256) for c in (0, 256)]
    for j, f in enumerate(beta_forms(*blk)):
      dst[j] = st_bf(f())

  def rows2(ref, r):
    return ref[pl.ds(r, H), :], ref[pl.ds(r + H, H), :]

  def init_quads(ref, r, cast=False):
    q = [ref[pl.ds(r + h, H), c:c + 256] for h in (0, H) for c in (0, 256)]
    return [v.astype(F32) for v in q] if cast else q

  def store_quads(ref, r, y):
    ref[pl.ds(r, H), :] = jnp.concatenate([y[0], y[1]], axis=1)
    ref[pl.ds(r + H, H), :] = jnp.concatenate([y[2], y[3]], axis=1)

  def store_tied(bd, ref, lead, r0, c0, val, step):
    for rr in range(0, val.shape[0], step):
      n = min(step, val.shape[0] - rr)
      ref[lead + (pl.ds(r0 + rr, n), slice(c0, c0 + val.shape[1]))] = val[rr:rr + n]
      got = ref[lead + (pl.ds(r0 + rr + n - 8, 8), slice(c0, c0 + 128))]
      bd.push([got if got.dtype == F32 else pltpu.bitcast(got, F32)], n * val.shape[1] // 1024)

  def ln_deps(ha, hb):
    return row_vregs(ha, 384) + row_vregs(hb, 384)

  class Body:
    def __init__(self, budget=BUDGET, nhi=25):
      self.nhi = nhi
      self.zm = zs[...] == 2
      self.budget = budget
      self.hi = []
      self.lo = []
      self.anchors = []

    def push(self, deps, w, hi=False):
      (self.hi if hi else self.lo).extend((w, 1, (lambda a, d=d: [d])) for d in deps)

    def push_lazy(self, w, n, fn):
      self.lo.append((w, n, fn))

    def note_result(self, r):
      self.anchors.append(r[0:8, 0:128])

    def gate(self, x, anchor):
      nr, nc = x.shape[0] // 8, x.shape[1] // 128
      return jnp.where(rep(rep(self.zm, nr, 0), nc, 1), rep(rep(anchor, nr, 0), nc, 1), x)

    def anchor(self):
      return self.anchors[-GATE] if GATE and len(self.anchors) >= GATE else None

    def take(self, budget, nhi, slots=50):
      out, tot = [], 0
      anchor = self.anchor()
      while self.hi and len(out) < nhi:
        w, n, fn = self.hi.pop(0)
        out += fn(anchor)
        tot += w * HIW
      while self.lo:
        w, n, fn = self.lo[0]
        if tot + w > budget or len(out) + n > slots:
          break
        self.lo.pop(0)
        tot += w
        out += fn(anchor)
      return out

    def flush_lo(self):
      anchor = self.anchor()
      rest = []
      for w, n, fn in self.lo:
        ds = fn(anchor)
        rest += [(w // max(n, 1), 1, (lambda a, d=d: [d])) for d in ds]
      self.lo = rest

    def flush(self):
      chain = [self.anchor()]
      for _, n, fn in self.hi + self.lo:
        out = fn(chain[-FLD] if len(chain) >= FLD else chain[0])
        if n > 1:
          chain.append(out[0])
      self.hi, self.lo = [], []

    def lhs_u(self, u, budget):
      return ld_bf(tie(self.zm, u, self.take(budget, self.nhi), True))

    def lhs_f(self, x, budget):
      return tie(self.zm, x, self.take(budget, NHIF if budget else 0, 2 * (x.shape[0] // 8)), False).astype(BF)

  def producer_thunks(bd, gam, get_u, rhs_fn, nt_dims, order=AORD, nhf=2):
    def mk(j):
      def run_():
        u = get_u(j)
        outs = []
        for hf in range(nhf):
          lhs = bd.lhs_u(u(hf), bd.budget)
          rhs = rhs_fn(j, hf)
          outs.append(dot_nt(lhs, rhs) if nt_dims else dot(lhs, rhs))
          bd.note_result(outs[-1])
        gam.add(j, jnp.concatenate(outs, axis=1) if nhf > 1 else outs[0])
      return run_
    return [mk(j) for j in order]

  def consumer_thunks(bd, gam, forms, rhs_fn, budget=0, order=BORD, cache=None):
    def mk(j):
      def run_():
        if cache is not None and j in cache:
          lv = cache[j]
        else:
          lv = bd.lhs_f(forms[j](), budget)
          if cache is not None:
            cache[j] = lv
        res = dot(lv, rhs_fn(j))
        bd.note_result(res)
        gam.add(j, res)
      return run_
    return [mk(j) for j in order]

  def scratch_u(j):
    return lambda hf: qa[j]

  def fresh_u(forms):
    def get(j):
      u = st_bf(forms[j]())
      qa[j] = u
      return lambda hf: u if hf == 0 else qa[j]
    return get

  def run(thunks):
    for th in thunks:
      th()

  def ff_act(bd, p, skip=()):
    def cb(q, z):
      if q in skip:
        p[q] = z
        return
      u = half_silu(z)
      p[q] = u
      bd.push(row_vregs(jnp.maximum(jnp.maximum(u[:, 0:128], u[:, 128:256]),
                                    jnp.maximum(u[:, 256:384], u[:, 384:512]))), 20, hi=True)
    return cb

  def ff_carried(bd):
    p = [sS[0], sS[1], sS[2], None]
    ff_act(bd, p)(3, sS[3])
    return p

  def ff_a(bd, gz, get_u, cn):
    return producer_thunks(bd, gz, get_u,
                           lambda j, hf: ld_bf(WA[j, :, cn * 512 + hf * 256:cn * 512 + hf * 256 + 256]), False)

  def ff_b(bd, gy, p, c):
    return consumer_thunks(bd, gy, alpha_forms(*p), lambda j: ld_bf(WB[j, c * 256:(c + 1) * 256, :]))

  def ff_step(bd, c, p, get_u, cn, gy, act, extra=None):
    pn = [None] * 4
    gz = Gamma(on_final=ff_act(bd, pn, () if act else (3,)))
    seq = interleave(ff_a(bd, gz, get_u, cn), ff_b(bd, gy, p, c))
    if extra is not None:
      seq[extra[0]:extra[0]] = extra[1]
    run(seq)
    return pn

  class LazyLN:
    def __init__(self, bd, load, front=False):
      self.bd = bd
      self.out = [[None] * (H // LNR), [None] * (H // LNR)]
      self.todo = []
      items = []
      for i in range(H // LNR):
        for h in range(2):
          def fn(anchor, h=h, i=i):
            if self.out[h][i] is None:
              x = load(h, i * LNR)
              if anchor is not None and LNGATE:
                x = bd.gate(x, anchor)
              self.out[h][i] = ln_rows(x)
            return row_vregs(self.out[h][i], 384)
          self.todo.append(fn)
          items.append((W_LN * (LNR // 8), LNR // 8, fn))
      if front:
        bd.lo[0:0] = items
      else:
        bd.lo.extend(items)

    def get(self):
      for fn in self.todo:
        fn(None)
      return [jnp.concatenate(v, axis=0) for v in self.out]

  def post_g(bd, t):
    r = mult(t * TM, TM)
    ln = LazyLN(bd, lambda h, r0: x1[pl.ds(r + h * H + r0, LNR), :])
    b = t // TPB
    rq_ = mult((t % TPB) * (H // 2), H // 2)
    forms = []

    def group(j, lo_, hi_, anchor):
      if not forms:
        forms.extend(alpha_forms(*quads(*ln.get())))
      f = forms[j]()[2 * lo_:2 * hi_]
      if anchor is not None:
        f = bd.gate(f, anchor)
      v = st_bf(f)
      G[b, j, pl.ds(rq_ + lo_, hi_ - lo_), :] = v
      got = G[b, j, pl.ds(rq_ + hi_ - 8, 8), 0:128]
      return [pltpu.bitcast(v[r_:r_ + 8, 128:256], F32) for r_ in range(0, hi_ - lo_, 16)] + [pltpu.bitcast(got, F32)]

    for j in range(7):
      for lo_, hi_ in ((0, 104), (104, 200)):
        bd.push_lazy(W_G * (hi_ - lo_) // 8, (hi_ - lo_ + 15) // 16 + 1,
                     lambda a, j=j, lo_=lo_, hi_=hi_: group(j, lo_, hi_, a))

  def qp_thunks(bd, gq, t):
    b = t // TPB
    rn = mult((t % TPB) * (H // 2), H // 2)
    return producer_thunks(bd, gq, lambda j: (lambda hf: G[b, j, pl.ds(rn, H // 2), :]),
                           lambda j, hf: ld_bf(MQK[j]), False, nhf=1)

  def s_thunks(bd, gs, get_u, b, c):
    return producer_thunks(bd, gs, get_u,
                           lambda j, hf: ld_bf(G[b, j, c * 256 + hf * 128:c * 256 + (hf + 1) * 128, :]),
                           True, order=TORD)

  class Att:
    def __init__(self):
      self.m = [None, None]
      self.l = [None, None]
      self.al = [None, None]
      self.acc = None

  def soft_cb(bd, at, c, p):
    held = {}

    def cb(q, sv):
      if c == 3:
        col = jax.lax.broadcasted_iota(jnp.int32, (H, 512), 1)
        sv = jnp.where(col < 512 - 48, sv, NEG)
      if q in (0, 2):
        held[q] = sv
        return
      hh = q // 2
      sa, sb = held[q - 1], sv
      mx = jnp.max(jnp.maximum(sa, sb), axis=-1, keepdims=True)
      mo = at.m[hh]
      mn = mx if mo is None else jnp.maximum(mo, mx)
      pa, pb = jnp.exp2(sa - mn), jnp.exp2(sb - mn)
      ta, tb = [(u[:, 0:128] + u[:, 128:256]) + (u[:, 256:384] + u[:, 384:512]) for u in (pa, pb)]
      if mo is None:
        at.al[hh] = None
        at.l[hh] = ta + tb
      else:
        at.al[hh] = jnp.exp2(mo - mn)
        at.l[hh] = at.l[hh] * at.al[hh] + (ta + tb)
      at.m[hh] = mn
      p[q - 1], p[q] = pa, pb
      for t_ in ((ta, tb) if hh == 0 else (tb, ta)):
        bd.push(row_vregs(t_), 12, hi=True)
      if c < 3:
        bd.push(row_vregs(at.l[hh]), 4, hi=True)
    return cb

  def att_carried(bd, at):
    p = [None] * 4
    cb = soft_cb(bd, at, 0, p)
    for q in range(4):
      cb(q, sS[q])
    return p

  def att_step(bd, at, b, c, p, get_u, bn_, cn, act=True, pv_budget=0):
    if at.acc is None:
      go = Gamma()
    else:
      acc = at.acc
      go = Gamma([(lambda q=q: acc[q] * al[q // 2]) for q in range(4)])
    al = list(at.al)
    pv = consumer_thunks(bd, go, alpha_forms(*p), lambda j: ld_bf(G[b, PVMAP[j], c * 256:(c + 1) * 256, :]),
                         budget=pv_budget)
    res = None
    if get_u is not None:
      pn = [None] * 4
      gs = Gamma(transposed=True, on_final=soft_cb(bd, at, cn, pn) if act else None)
      run(interleave(s_thunks(bd, gs, get_u, bn_, cn), pv))
      res = pn if act else gs.result()
    else:
      run(pv)
    at.acc = go.result()
    return res

  LS = TM // 8

  def conv_outputs(U, ls, dwk, u0, u1):
    start = (U % TPB) == 0
    win = {}

    def inp(u):
      if u not in win:
        win[u] = gb[ls, pl.ds(8 + u, 8, stride=LS), :]
      return win[u]

    outs = []
    for u in range(u0, u1):
      acc = [None, None]
      for k in range(KW):
        ui = u + k - KW // 2
        v = inp(ui)
        if start and u < 15 and ((u < 8) != (ui < 8)):
          v = jnp.where(sub0, 0.0, v)
        t = v * dwk[k]
        acc[k & 1] = t if acc[k & 1] is None else acc[k & 1] + t
      outs.append(acc[0] + acc[1])
    return outs

  def conv_unit(bd, U, lanes=(0, 1, 2, 3)):
    ru = (U + 1) * TM
    bounds = [(LS * g + NG // 2) // NG for g in range(NG + 1)]

    def make(l):
      ls = slice(l * 128, (l + 1) * 128)
      state = {}

      def group(g, anchor):
        u0, u1 = bounds[g], bounds[g + 1]
        dwk = [DWB[k, :, ls] for k in range(KW)]
        if anchor is not None:
          dwk = [bd.gate(v, anchor) for v in dwk]
        outs = conv_outputs(U, l, dwk, u0, u1)
        if g == 0:
          if U == 0:
            st[0:8, ls] = outs[8]
          state["k"] = outs[8] if U == 0 else st[0:8, ls]
          state["s1"] = st[8:16, ls]
          state["s2"] = st[16:24, ls]
        deps = []
        for u, o in zip(range(u0, u1), outs):
          d = o - state["k"]
          if U == 0 and u < 8:
            d = jnp.where(sub0, 0.0, d)
          d2 = d * d
          state["s1"] = state["s1"] + d
          state["s2"] = state["s2"] + d2
          dc[l, pl.ds(ru + u, 8, stride=LS), :] = o
          deps.append(d2)
        deps.append(dc[l, pl.ds(ru + u1 - 1, 8, stride=LS), :])
        if g == NG - 1:
          st[8:16, ls] = state["s1"]
          st[16:24, ls] = state["s2"]
        return deps
      return group

    for l in lanes:
      grp = make(l)
      for g in range(NG):
        n = bounds[g + 1] - bounds[g]
        bd.push_lazy(W_CONV * n + 15, n + 1, lambda a, grp=grp, g=g: grp(g, a))

  def conv_part(win, nr, dwk):
    acc = [None, None]
    for rho in range(8):
      if rho == 0:
        tt = win[8:8 + nr] * rep(dwk[7], nr // 8, 0)
      else:
        u = (win[0:nr + 8] * rep(dwk[rho - 1], nr // 8 + 1, 0)
             + win[8:nr + 16] * rep(dwk[rho + 7], nr // 8 + 1, 0))
        tt = pltpu.roll(u, nr + 8 - rho, 0)[0:nr]
      acc[rho & 1] = tt if acc[rho & 1] is None else acc[rho & 1] + tt
    return acc[0] + acc[1]

  def conv_exposed(bd, U, lanes):
    keep = bd.hi, bd.lo
    bd.hi, bd.lo = [], []
    conv_unit(bd, U, lanes)
    for _, _, fn in bd.lo:
      fn(None)
    bd.hi, bd.lo = keep

  def conv_tail(lanes):
    for l in lanes:
      ls = slice(l * 128, (l + 1) * 128)
      dwk = [DWB[k, :, ls] for k in range(KW)]
      halo = gb[l, TM:TM + 16, :]
      w = jnp.concatenate([halo, jnp.zeros((8, 128), F32)], axis=0)
      out = conv_part(w, 8, dwk)
      dc[l, N + TM:N + TM + 8, :] = out
      d = out - st[0:8, ls]
      st[8:16, ls] = st[8:16, ls] + d
      st[16:24, ls] = st[16:24, ls] + d * d

  def epi_mvo(bd, t, budget=0):
    r = mult(t * TM, TM)
    rl = [1.0 / jnp.sum(lsc[hh], axis=-1, keepdims=True) for hh in range(2)]
    oq = [osc[0] * rl[0], osc[1] * rl[0], osc[2] * rl[1], osc[3] * rl[1]]
    g = Gamma(init_quads(x1, r))
    run(consumer_thunks(bd, g, alpha_forms(*oq), lambda j: ld_bf(MVO[j]), budget=budget))
    y = g.result()
    xs = [jnp.concatenate([y[0], y[1]], axis=1), jnp.concatenate([y[2], y[3]], axis=1)]
    for h, v in zip((0, H), xs):
      store_tied(bd, x1, (), r + h, 0, v, 80)
    return [ln_rows(v) for v in xs]

  def epi_pw1(bd, ha, hb, sl, cache, budget=0, pre_store=None):
    g = Gamma()
    run(consumer_thunks(bd, g, alpha_forms(*quads(ha, hb)),
                        lambda j: ld_bf(WP1[j, :, sl * 256:(sl + 1) * 256]), order=AORD, cache=cache,
                        budget=budget))
    if pre_store is not None:
      pre_store()
    a1, b1, a2, b2 = g.result()
    deps = []
    for h, gv in ((0, a1 + a1 * jnp.tanh(b1)), (H, a2 + a2 * jnp.tanh(b2))):
      for k in range(2):
        gb[2 * sl + k, 16 + h:16 + h + H, :] = gv[:, k * 128:(k + 1) * 128]
        deps += [gb[2 * sl + k, r:r + 8, :] for r in range(16 + h, 16 + h + H, 8)]
    return deps

  def pre3(bd, t):
    r = mult(t * TM, TM)
    mu = rep(bn[0:8, :], H // 8, 0)
    hrs = rep(bn[8:16, :], H // 8, 0)
    hs = [half_silu((jnp.concatenate([dc[l, pl.ds(r + TM + 8 + h, H), :] for l in range(4)], axis=1)
                     - mu) * hrs) for h in (0, H)]
    for u in hs:
      bd.push(row_vregs(jnp.maximum(jnp.maximum(u[:, 0:128], u[:, 128:256]),
                                    jnp.maximum(u[:, 256:384], u[:, 384:512]))), 24, hi=True)
    g = Gamma(init_quads(x1, r))
    holder = []

    def finish():
      y = g.result()
      xs = [jnp.concatenate([y[0], y[1]], axis=1), jnp.concatenate([y[2], y[3]], axis=1)]
      ha, hb = [ln_rows(v) for v in xs]
      bd.lo[0:0] = [(W_LN, 1, (lambda a, d=d: [d])) for d in ln_deps(ha, hb)]
      for h, v in zip((0, H), xs):
        store_tied(bd, x1, (), r + h, 0, v, 80)
      holder.extend([ha, hb])

    return consumer_thunks(bd, g, alpha_forms(*quads(*hs)), lambda j: ld_bf(WP2[j])) + [finish], holder

  def post3(bd, t):
    r = mult(t * TM, TM)

    def piece(r0, anchor):
      x = x1[pl.ds(r + r0, LNR), :]
      if anchor is not None and LNGATE:
        x = bd.gate(x, anchor)
      o = ln_rows(x)
      xo[pl.ds(r + r0, LNR), :] = o.astype(BF)
      got = pltpu.bitcast(xo[pl.ds(r + r0 + LNR - 16, 16), 0:128], U32)
      return row_vregs(o, 384) + [pltpu.bitcast(got, F32)]

    for r0 in range(0, TM, LNR):
      bd.push_lazy((W_LN + 4) * (LNR // 8), LNR // 8 + 1, lambda a, r0=r0: piece(r0, a))

  sub0 = jax.lax.broadcasted_iota(jnp.int32, (8, 128), 0) == 0

  def zero_step(j, c):
    for b in range(NB):
      G[b, j, T // 4:1024, :] = jnp.zeros((1024 - T // 4, 256), U32)
    return c
  jax.lax.fori_loop(0, 7, zero_step, 0)

  def zero_rows(i, c):
    r = mult(i * 48, 8)
    gb[:, pl.ds(r, 48), :] = jnp.zeros((4, 48, 128), F32)
    x1[pl.ds(r, 48), :] = jnp.zeros((48, D), F32)
    return c
  jax.lax.fori_loop(0, (TM + 16) // 48, zero_rows, 0)
  st[...] = jnp.zeros(st.shape, F32)

  wcopy(I_Q).wait()
  wcopy(I_K).wait()
  prep_from_value(dot_nt(rq[...], rk[...]) * QSCALE, MQK)
  wcopy(I_V).wait()
  wcopy(I_O).wait()
  wcopy(I_B1).start()
  xcopy(1).start()
  prep_from_value(dot(rv[...], ro[...]), MVO)
  xcopy(0).wait()
  zs[...] = pltpu.bitcast(xo[0:16, 0:128], U32) >> 31
  wcopy(I_A1).wait()

  def prep_wa1(i, c):
    c0 = mult(i * 256, 256)
    blk = [ra1[r:r + 256, pl.ds(c0 + cc, 256)].astype(F32) * 0.5 for r in (0, 256) for cc in (0, 1024)]
    for j, f in enumerate(beta_forms(*blk)):
      WA[j, :, pl.ds(c0, 256)] = st_bf(f())
    return c
  jax.lax.fori_loop(0, 4, prep_wa1, 0)
  bd = Body()
  ha, hb = [ln_rows(v.astype(F32)) for v in rows2(xo, 0)]
  wcopy(I_B1).wait()
  for t in range(2, NT):
    xcopy(t).start()
  for i in (I_P1, I_DW, I_P2, I_A2, I_B2):
    wcopy(i).start()
  bd.push(prep_weight(rb1, WB, 1024, 256, 0.5), W_PREP)
  gz = Gamma()
  run(ff_a(bd, gz, fresh_u(alpha_forms(*quads(ha, hb))), 0))
  for k, v in enumerate(gz.result()):
    sS[k] = half_silu(v) if k < 3 else v

  def p1_body(t, last):
    bd = Body(BUD1, NHI1)
    r0 = mult(t * TM, TM)
    if not last:
      xcopy(t + 1).wait()
      rn = mult((t + 1) * TM, TM)
      lnx = LazyLN(bd, lambda h, r0: xo[pl.ds(rn + h * H + r0, LNR), :].astype(F32))
    post_g(bd, max(t - 1, 0) if isinstance(t, int) else jnp.maximum(t - 1, 0))
    gy = Gamma(init_quads(xo, r0, cast=True), reps=2)
    p = ff_step(bd, 0, ff_carried(bd), scratch_u, 1, gy, True)
    if not last:
      z = ff_step(bd, 1, p, fresh_u(alpha_forms(*quads(*lnx.get()))), 0, gy, False)
      store_quads(x1, r0, gy.result())
      for k in range(4):
        sS[k] = z[k]
    else:
      bth = ff_b(bd, gy, p, 1)
      gq = Gamma()
      run(merge(qp_thunks(bd, gq, 0), bth[:3]))
      gs = Gamma(transposed=True)
      run(merge(s_thunks(bd, gs, fresh_u(phi_forms(*gq.result())), 0, 0), bth[3:]))
      store_quads(x1, r0, gy.result())
      for k, v in enumerate(gs.result()):
        sS[k] = v
    bd.flush()

  if 'P1' in PHASES:
    jax.lax.fori_loop(0, NT - 1, lambda t, c: (p1_body(t, False), c)[1], 0)
  else:
    for t in range(1, NT):
      xcopy(t).wait()
  if 'P1L' in PHASES:
    p1_body(NT - 1, True)

  def p2_body(i, first, last):
    bd = Body(BUD2, NHI2)
    b = i // TPB
    bn_ = (i + 1) // TPB
    at = Att()
    if first:
      for k in (I_P1, I_DW, I_P2, I_A2, I_B2):
        wcopy(k).wait()
      post_g(bd, NT - 1)
      dwf = rdw[...].astype(F32)
      for k in range(KW):
        DWB[k] = jnp.broadcast_to(dwf[k:k + 1, :], (8, D))
      bd.push(prep_weight(rp1, WP1, 256, 512, 0.5), W_PREP)
      bd.push(prep_weight(rp2, WP2, 256, 256, 1.0), W_PREP)
      bd.push(prep_weight(ra2, WA, 256, 1024, 0.5), W_PREP)
      bd.push(prep_weight(rb2, WB, 1024, 256, 0.5), W_PREP)
    else:
      conv_unit(bd, i - 2)
      halo = gb[:, TM:TM + 16, :]
    s = att_step(bd, at, b, 0, att_carried(bd, at), scratch_u, b, 1)
    if not first:
      ha, hb = epi_mvo(bd, i - 1, budget=BUDM)
    s = att_step(bd, at, b, 1, s, scratch_u, b, 2)
    if not first:
      bd.push(ln_deps(ha, hb), W_LN)
    s = att_step(bd, at, b, 2, s, scratch_u, b, 3)
    if not first:
      cache = {}

      def roll_window():
        bd.flush_lo()
        gb[:, 0:16, :] = halo

      gd = epi_pw1(bd, ha, hb, 0, cache, budget=BUDP, pre_store=roll_window)
      gd += epi_pw1(bd, ha, hb, 1, cache)
      if not last:
        bd.push(gd, 8)
    if not last:
      gq = Gamma()
      run(qp_thunks(bd, gq, i + 1))
      s = att_step(bd, at, b, 3, s, fresh_u(phi_forms(*gq.result())), bn_, 0, False)
      for k in range(4):
        sS[k] = s[k]
    else:
      conv_unit(bd, i - 1, HOST8)
      att_step(bd, at, b, 3, s, None, None, None, pv_budget=BUDL)
    for k in range(4):
      osc[k] = at.acc[k]
    for hh in range(2):
      lsc[hh] = at.l[hh]
    if first:
      bd.flush()
    return bd

  if 'P2F' in PHASES:
    p2_body(0, True, False)
  else:
    for k in (I_P1, I_DW, I_P2, I_A2, I_B2):
      wcopy(k).wait()
  def p2_pair(k, c):
    p2_body(2 * k + 1, False, False)

    @pl.when(k >= 0)
    def _():
      p2_body(2 * k + 2, False, False)
    return c
  if 'P2' in PHASES:
    for i_ in range(1, P2N):
      if BOUND == 'when':
        pl.when(z_s[0] == 0)(lambda i_=i_: p2_body(i_, False, False) and None)
      else:
        p2_body(i_, False, False)
        if BOUND == 'delay':
          pl.delay(1)
  if 'P2S' in PHASES:
    pl.when(z_s[0] == 0)(lambda: p2_body(3, False, False) and None)
  if 'P2L' in PHASES:
    bd = p2_body(NT - 1, False, True)
  else:
    bd = Body()
    conv_unit(bd, NT - 2, HOST8)

  ha, hb = epi_mvo(bd, NT - 1, budget=BUDL2)

  def roll_window():
    print("leftover groups", len(bd.lo)) if DEBUG else None
    bd.flush()
    conv_exposed(bd, NT - 2, [l for l in range(4) if l not in HOST8])
    gb[:, 0:16, :] = gb[:, TM:TM + 16, :]

  epi_pw1(bd, ha, hb, 0, None, budget=BUDL2, pre_store=roll_window)
  conv_unit(bd, NT - 1, HOSTL)
  epi_pw1(bd, ha, hb, 1, None, budget=BUDL3)
  bd.flush()
  conv_exposed(bd, NT - 1, [l for l in range(4) if l not in HOSTL])
  conv_tail((0, 1, 2, 3))
  n_s = jnp.where(jax.lax.broadcasted_iota(jnp.int32, (8, D), 0) == 0, N // 8 - 7.0, N // 8 + 1.0)
  s1 = st[8:16, :]
  mu_s = st[0:8, :] + s1 / n_s
  m2_s = st[16:24, :] - s1 * s1 / n_s
  mu = jnp.sum(mu_s * n_s, axis=0, keepdims=True) * (1.0 / N)
  dm = mu_s - mu
  var = jnp.sum(m2_s + dm * dm * n_s, axis=0, keepdims=True) * (1.0 / N)
  bn[0:8, :] = jnp.broadcast_to(mu, (8, D))
  bn[8:16, :] = jnp.broadcast_to(0.5 * jax.lax.rsqrt(var + EPS), (8, D))

  bd = Body()
  th, (hold) = pre3(bd, 0)
  run(th)
  ha, hb = hold
  gz = Gamma()
  run(ff_a(bd, gz, fresh_u(alpha_forms(*quads(ha, hb))), 0))
  for k, v in enumerate(gz.result()):
    sS[k] = half_silu(v) if k < 3 else v

  def p3_body(t, last):
    bd = Body(BUD3, NHI3)
    r0 = mult(t * TM, TM)

    @pl.when(t >= 2)
    def _():
      ocopy(t - 2).start()

    p0 = ff_carried(bd)
    extra = None
    if not last:
      th, hold = pre3(bd, t + 1)
      extra = (P3POS, th)
    post3(bd, max(t - 1, 0) if isinstance(t, int) else jnp.maximum(t - 1, 0))
    gy = Gamma(init_quads(x1, r0), reps=2)
    p = ff_step(bd, 0, p0, scratch_u, 1, gy, True, extra)
    if not last:
      z = ff_step(bd, 1, p, fresh_u(alpha_forms(*quads(*hold))), 0, gy, False)
      for k in range(4):
        sS[k] = z[k]
    else:
      run(ff_b(bd, gy, p, 1))
    store_quads(x1, r0, gy.result())
    bd.flush()

  if 'P3' in PHASES:
    jax.lax.fori_loop(0, NT - 1, lambda t, c: (p3_body(t, False), c)[1], 0)
  if 'P3L' in PHASES:
    p3_body(NT - 1, True)

  bd = Body()
  ocopy(NT - 2).start()
  post3(bd, NT - 1)
  bd.flush()
  ocopy(NT - 1).start()
  for t in range(NT):
    ocopy(t).wait()


@jax.jit
def pallas_standalone__conformer_family_conformer__speech_kernel(
    x, w_ff1_a, w_ff1_b, w_q, w_k, w_v, w_o, w_pw1, dw, w_pw2, w_ff2_a, w_ff2_b):
  hbm = pl.BlockSpec(memory_space=pl.ANY)
  V = pltpu.VMEM
  out = pl.pallas_call(
      kernel,
      out_shape=jax.ShapeDtypeStruct((N, D), x.dtype),
      in_specs=[pl.BlockSpec(memory_space=pltpu.SMEM)] + [hbm] * 12,
      out_specs=hbm,
      scratch_shapes=[
          V((N, D), BF),
          V((D, FH), BF), V((FH, D), BF), V((D, FH), BF), V((FH, D), BF),
          V((D, D), BF), V((D, D), BF), V((D, D), BF), V((D, D), BF),
          V((D, 2 * D), BF), V((KW, D), BF), V((D, D), BF),
          V((7, 128, 1024), U32), V((7, 512, 256), U32),
          V((7, 128, 256), U32), V((7, 128, 256), U32),
          V((7, 128, 512), U32), V((7, 128, 256), U32),
          V((KW, 8, D), F32),
          V((N, D), F32),
          V((4, N + TM + 8, 128), F32),
          V((NB, 7, 1024, 256), U32),
          V((4, TM + 16, 128), F32),
          V((4, H, 512), F32),
          V((7, H // 2, 256), U32),
          V((4, H, 256), F32),
          V((2, H, 128), F32),
          V((24, D), F32), V((16, D), F32), V((8, 128), U32),
          pltpu.SemaphoreType.DMA((2 * NT + 11,)),
      ],
      compiler_params=pltpu.CompilerParams(vmem_limit_bytes=124 * 1024 * 1024),
  )(jnp.zeros((1,), jnp.int32), x.reshape(N, D), w_ff1_a, w_ff1_b, w_q, w_k, w_v, w_o, w_pw1, dw, w_pw2, w_ff2_a, w_ff2_b)
  return out.reshape(NB, T, D)
```

```python
import jax
import jax.numpy as jnp
import jax.experimental.pallas as pl
import jax.experimental.pallas.tpu as pltpu

BF = jnp.bfloat16
F32 = jnp.float32
U32 = jnp.uint32

NB, T, D, FH, KW = 2, 4000, 512, 2048, 15
N = NB * T
TM = 800
H = TM // 2
NT = N // TM
TPB = T // TM
EPS = 1e-5
QSCALE = D ** -0.5 * 1.4426950408889634
NEG = -1e30

PVMAP = [0, 2, 6, 5, 3, 4, 1]
AORD = [0, 3, 4, 6, 2, 1, 5]
TORD = [0, 3, 4, 6, 1, 2, 5]
BORD = [2, 4, 0, 3, 6, 5, 1]
W_LN, W_PREP = 36, 9
BUD1, BUD2, BUD3, BUDM = 800, 700, 1000, 700
NHI1, NHI2, NHI3 = 35, 34, 35
NHI, NHIF, HIW, GATE, NG = 40, 0, 1, 2, 6
P3POS = 6
BUDL, BUDL2, BUDL3 = 1500, 850, 850
FLD = 2
BUDP = 850
HOSTL = (0,)
HOST8 = (0, 1, 2)
W_CONV = 36
LNR, LNGATE, W_G = 80, True, 22
BUDGET = 560
CONTRIB = [((0, 1), (3, 1)), ((2, 1), (3, -1)), ((1, 1), (3, 1)), ((0, 1), (2, 1)),
           ((0, -1), (1, 1)), ((3, 1),), ((0, 1),)]


def dot(a, b):
  return jnp.dot(a, b, preferred_element_type=F32)


def dot_nt(a, b):
  return jax.lax.dot_general(a, b, (((1,), (1,)), ((), ())), preferred_element_type=F32)


def alpha_forms(a11, a12, a21, a22):
  return [lambda: a11 + a22, lambda: a21 + a22, lambda: a11, lambda: a22,
          lambda: a11 + a12, lambda: a21 - a11, lambda: a12 - a22]


def beta_forms(b11, b12, b21, b22):
  return [lambda: b11 + b22, lambda: b11, lambda: b12 - b22, lambda: b21 - b11,
          lambda: b22, lambda: b11 + b12, lambda: b21 + b22]


def phi_forms(q11, q12, q21, q22):
  return beta_forms(q11, q21, q12, q22)


def quads(ha, hb):
  return ha[:, :256], ha[:, 256:], hb[:, :256], hb[:, 256:]


class Gamma:
  def __init__(self, init=None, transposed=False, on_final=None, reps=1):
    self.p = [None] * 4 if init is None else list(init)
    self.sg = [1] * 4
    self.left = [4 * reps, 2 * reps, 2 * reps, 4 * reps]
    self.tr = transposed
    self.on_final = on_final

  def add(self, j, m):
    for q, sg in CONTRIB[j]:
      if self.tr and q in (1, 2):
        q = 3 - q
      v = self.p[q]
      if callable(v):
        v = v()
      s = self.sg[q]
      if v is None:
        self.p[q], self.sg[q] = m, sg
      elif s == 1:
        self.p[q] = v + m if sg == 1 else v - m
      else:
        self.p[q], self.sg[q] = (m - v, 1) if sg == 1 else (v + m, -1)
      self.left[q] -= 1
      if self.left[q] == 0:
        assert self.sg[q] == 1
        if self.on_final is not None:
          self.on_final(q, self.p[q])

  def result(self):
    assert all(n == 0 for n in self.left)
    return list(self.p)


def rep(x, n, axis):
  return jnp.concatenate([x] * n, axis=axis) if n > 1 else x


def ld_bf(u):
  return pltpu.bitcast(u, BF)


def st_bf(x):
  return pltpu.bitcast(x.astype(BF), U32)


def ln_rows(x):
  m = jnp.mean(x, axis=-1, keepdims=True)
  xc = x - m
  v = jnp.mean(xc * xc, axis=-1, keepdims=True)
  return xc * jax.lax.rsqrt(v + EPS)


def half_silu(hz):
  return hz + hz * jnp.tanh(hz)


def row_vregs(x, c0=0):
  return [x[r:r + 8, c0:c0 + 128] for r in range(0, x.shape[0], 8)]


def tie(zm, u, deps, cast):
  if not deps:
    return u
  n = u.shape[0] // 8
  nk = u.shape[1] // 128
  slots = n * nk
  assign = {}
  for idx, d in enumerate(deps):
    assign[(idx * slots) // len(deps)] = d
  rows = []
  for rb in range(n):
    blk = u[rb * 8:(rb + 1) * 8]
    if any((rb * nk + k) in assign for k in range(nk)):
      parts = []
      for k in range(nk):
        pc = blk[:, k * 128:(k + 1) * 128]
        d = assign.get(rb * nk + k)
        if d is not None:
          pc = jnp.where(zm, pltpu.bitcast(d, U32) if cast else d, pc)
        parts.append(pc)
      blk = jnp.concatenate(parts, axis=1)
    rows.append(blk)
  return jnp.concatenate(rows, axis=0)


def sel(c, a, b):
  if isinstance(c, bool):
    return a if c else b
  return jnp.where(c, a, b)


def mult(x, n):
  return x if isinstance(x, int) else pl.multiple_of(x, n)


def interleave(a, b):
  out = []
  for i in range(max(len(a), len(b))):
    if i < len(a):
      out.append(a[i])
    if i < len(b):
      out.append(b[i])
  return out


def merge(s1, s2):
  out, n1, n2, i, j = [], len(s1), len(s2), 0, 0
  while i < n1 or j < n2:
    if j >= n2 or (i < n1 and i * n2 <= j * n1):
      out.append(s1[i]); i += 1
    else:
      out.append(s2[j]); j += 1
  return out


def kernel(x_h, wa1_h, wb1_h, wq_h, wk_h, wv_h, wo_h, wp1_h, dw_h, wp2_h, wa2_h, wb2_h, out_h,
           xo, ra1, rb1, ra2, rb2, rq, rk, rv, ro, rp1, rdw, rp2,
           WA, WB, MQK, MVO, WP1, WP2, DWB, x1, dc, G, gb, sS, qa, osc, lsc, st, bn, zs, sem):

  def xcopy(t):
    return pltpu.make_async_copy(x_h.at[pl.ds(t * TM, TM)], xo.at[pl.ds(t * TM, TM)], sem.at[t])

  def ocopy(t):
    return pltpu.make_async_copy(xo.at[pl.ds(t * TM, TM)], out_h.at[pl.ds(t * TM, TM)], sem.at[NT + 11 + t])

  wsrc = [wa1_h, wb1_h, wq_h, wk_h, wv_h, wo_h, wp1_h, dw_h, wp2_h, wa2_h, wb2_h]
  wdst = [ra1, rb1, rq, rk, rv, ro, rp1, rdw, rp2, ra2, rb2]
  I_A1, I_B1, I_Q, I_K, I_V, I_O, I_P1, I_DW, I_P2, I_A2, I_B2 = range(11)

  def wcopy(i):
    return pltpu.make_async_copy(wsrc[i], wdst[i], sem.at[NT + i])

  for i in (I_Q, I_K, I_V, I_O):
    wcopy(i).start()
  xcopy(0).start()
  wcopy(I_A1).start()

  def prep_weight(raw, dst, kh, nh, scale, cw=256):
    deps = []
    for c0 in range(0, nh, cw):
      for r0 in range(0, kh, 256):
        blk = [raw[r:r + 256, c:c + cw].astype(F32) * scale
               for r in (r0, kh + r0) for c in (c0, nh + c0)]
        for j, f in enumerate(beta_forms(*blk)):
          dst[j, r0 // 2:r0 // 2 + 128, c0:c0 + cw] = st_bf(f())
        for j in range(7):
          v = dst[j, r0 // 2:r0 // 2 + 128, c0:c0 + cw]
          deps += [pltpu.bitcast(v[r:r + 8, c:c + 128], F32)
                   for r in range(0, 128, 8) for c in range(0, cw, 128)]
    return deps

  def prep_from_value(m, dst):
    blk = [m[r:r + 256, c:c + 256] for r in (0, 256) for c in (0, 256)]
    for j, f in enumerate(beta_forms(*blk)):
      dst[j] = st_bf(f())

  def rows2(ref, r):
    return ref[pl.ds(r, H), :], ref[pl.ds(r + H, H), :]

  def init_quads(ref, r, cast=False):
    q = [ref[pl.ds(r + h, H), c:c + 256] for h in (0, H) for c in (0, 256)]
    return [v.astype(F32) for v in q] if cast else q

  def store_quads(ref, r, y):
    ref[pl.ds(r, H), :] = jnp.concatenate([y[0], y[1]], axis=1)
    ref[pl.ds(r + H, H), :] = jnp.concatenate([y[2], y[3]], axis=1)

  def store_tied(bd, ref, lead, r0, c0, val, step):
    for rr in range(0, val.shape[0], step):
      n = min(step, val.shape[0] - rr)
      ref[lead + (pl.ds(r0 + rr, n), slice(c0, c0 + val.shape[1]))] = val[rr:rr + n]
      got = ref[lead + (pl.ds(r0 + rr + n - 8, 8), slice(c0, c0 + 128))]
      bd.push([got if got.dtype == F32 else pltpu.bitcast(got, F32)], n * val.shape[1] // 1024)

  def ln_deps(ha, hb):
    return row_vregs(ha, 384) + row_vregs(hb, 384)

  class Body:
    def __init__(self, budget=BUDGET, nhi=25):
      self.nhi = nhi
      self.zm = zs[...] == 2
      self.budget = budget
      self.hi = []
      self.lo = []
      self.anchors = []

    def push(self, deps, w, hi=False):
      (self.hi if hi else self.lo).extend((w, 1, (lambda a, d=d: [d])) for d in deps)

    def push_lazy(self, w, n, fn):
      self.lo.append((w, n, fn))

    def note_result(self, r):
      self.anchors.append(r[0:8, 0:128])

    def gate(self, x, anchor):
      nr, nc = x.shape[0] // 8, x.shape[1] // 128
      return jnp.where(rep(rep(self.zm, nr, 0), nc, 1), rep(rep(anchor, nr, 0), nc, 1), x)

    def anchor(self):
      return self.anchors[-GATE] if GATE and len(self.anchors) >= GATE else None

    def take(self, budget, nhi, slots=50):
      out, tot = [], 0
      anchor = self.anchor()
      while self.hi and len(out) < nhi:
        w, n, fn = self.hi.pop(0)
        out += fn(anchor)
        tot += w * HIW
      while self.lo:
        w, n, fn = self.lo[0]
        if tot + w > budget or len(out) + n > slots:
          break
        self.lo.pop(0)
        tot += w
        out += fn(anchor)
      return out

    def flush_lo(self):
      anchor = self.anchor()
      rest = []
      for w, n, fn in self.lo:
        ds = fn(anchor)
        rest += [(w // max(n, 1), 1, (lambda a, d=d: [d])) for d in ds]
      self.lo = rest

    def flush(self):
      chain = [self.anchor()]
      for _, n, fn in self.hi + self.lo:
        out = fn(chain[-FLD] if len(chain) >= FLD else chain[0])
        if n > 1:
          chain.append(out[0])
      self.hi, self.lo = [], []

    def lhs_u(self, u, budget):
      return ld_bf(tie(self.zm, u, self.take(budget, self.nhi), True))

    def lhs_f(self, x, budget):
      return tie(self.zm, x, self.take(budget, NHIF if budget else 0, 2 * (x.shape[0] // 8)), False).astype(BF)

  def producer_thunks(bd, gam, get_u, rhs_fn, nt_dims, order=AORD, nhf=2):
    def mk(j):
      def run_():
        u = get_u(j)
        outs = []
        for hf in range(nhf):
          lhs = bd.lhs_u(u(hf), bd.budget)
          rhs = rhs_fn(j, hf)
          outs.append(dot_nt(lhs, rhs) if nt_dims else dot(lhs, rhs))
          bd.note_result(outs[-1])
        gam.add(j, jnp.concatenate(outs, axis=1) if nhf > 1 else outs[0])
      return run_
    return [mk(j) for j in order]

  def consumer_thunks(bd, gam, forms, rhs_fn, budget=0, order=BORD, cache=None):
    def mk(j):
      def run_():
        if cache is not None and j in cache:
          lv = cache[j]
        else:
          lv = bd.lhs_f(forms[j](), budget)
          if cache is not None:
            cache[j] = lv
        res = dot(lv, rhs_fn(j))
        bd.note_result(res)
        gam.add(j, res)
      return run_
    return [mk(j) for j in order]

  def scratch_u(j):
    return lambda hf: qa[j]

  def fresh_u(forms):
    def get(j):
      u = st_bf(forms[j]())
      qa[j] = u
      return lambda hf: u if hf == 0 else qa[j]
    return get

  def run(thunks):
    for th in thunks:
      th()

  def ff_act(bd, p, skip=()):
    def cb(q, z):
      if q in skip:
        p[q] = z
        return
      u = half_silu(z)
      p[q] = u
      bd.push(row_vregs(jnp.maximum(jnp.maximum(u[:, 0:128], u[:, 128:256]),
                                    jnp.maximum(u[:, 256:384], u[:, 384:512]))), 20, hi=True)
    return cb

  def ff_carried(bd):
    p = [sS[0], sS[1], sS[2], None]
    ff_act(bd, p)(3, sS[3])
    return p

  def ff_a(bd, gz, get_u, cn):
    return producer_thunks(bd, gz, get_u,
                           lambda j, hf: ld_bf(WA[j, :, cn * 512 + hf * 256:cn * 512 + hf * 256 + 256]), False)

  def ff_b(bd, gy, p, c):
    return consumer_thunks(bd, gy, alpha_forms(*p), lambda j: ld_bf(WB[j, c * 256:(c + 1) * 256, :]))

  def ff_step(bd, c, p, get_u, cn, gy, act, extra=None):
    pn = [None] * 4
    gz = Gamma(on_final=ff_act(bd, pn, () if act else (3,)))
    seq = interleave(ff_a(bd, gz, get_u, cn), ff_b(bd, gy, p, c))
    if extra is not None:
      seq[extra[0]:extra[0]] = extra[1]
    run(seq)
    return pn

  class LazyLN:
    def __init__(self, bd, load, front=False):
      self.bd = bd
      self.out = [[None] * (H // LNR), [None] * (H // LNR)]
      self.todo = []
      items = []
      for i in range(H // LNR):
        for h in range(2):
          def fn(anchor, h=h, i=i):
            if self.out[h][i] is None:
              x = load(h, i * LNR)
              if anchor is not None and LNGATE:
                x = bd.gate(x, anchor)
              self.out[h][i] = ln_rows(x)
            return row_vregs(self.out[h][i], 384)
          self.todo.append(fn)
          items.append((W_LN * (LNR // 8), LNR // 8, fn))
      if front:
        bd.lo[0:0] = items
      else:
        bd.lo.extend(items)

    def get(self):
      for fn in self.todo:
        fn(None)
      return [jnp.concatenate(v, axis=0) for v in self.out]

  def post_g(bd, t):
    r = mult(t * TM, TM)
    ln = LazyLN(bd, lambda h, r0: x1[pl.ds(r + h * H + r0, LNR), :])
    b = t // TPB
    rq_ = mult((t % TPB) * (H // 2), H // 2)
    forms = []

    def group(j, lo_, hi_, anchor):
      if not forms:
        forms.extend(alpha_forms(*quads(*ln.get())))
      f = forms[j]()[2 * lo_:2 * hi_]
      if anchor is not None:
        f = bd.gate(f, anchor)
      v = st_bf(f)
      G[b, j, pl.ds(rq_ + lo_, hi_ - lo_), :] = v
      got = G[b, j, pl.ds(rq_ + hi_ - 8, 8), 0:128]
      return [pltpu.bitcast(v[r_:r_ + 8, 128:256], F32) for r_ in range(0, hi_ - lo_, 16)] + [pltpu.bitcast(got, F32)]

    for j in range(7):
      for lo_, hi_ in ((0, 104), (104, 200)):
        bd.push_lazy(W_G * (hi_ - lo_) // 8, (hi_ - lo_ + 15) // 16 + 1,
                     lambda a, j=j, lo_=lo_, hi_=hi_: group(j, lo_, hi_, a))

  def qp_thunks(bd, gq, t):
    b = t // TPB
    rn = mult((t % TPB) * (H // 2), H // 2)
    return producer_thunks(bd, gq, lambda j: (lambda hf: G[b, j, pl.ds(rn, H // 2), :]),
                           lambda j, hf: ld_bf(MQK[j]), False, nhf=1)

  def s_thunks(bd, gs, get_u, b, c):
    return producer_thunks(bd, gs, get_u,
                           lambda j, hf: ld_bf(G[b, j, c * 256 + hf * 128:c * 256 + (hf + 1) * 128, :]),
                           True, order=TORD)

  class Att:
    def __init__(self):
      self.m = [None, None]
      self.l = [None, None]
      self.al = [None, None]
      self.acc = None

  def soft_cb(bd, at, c, p):
    held = {}

    def cb(q, sv):
      if c == 3:
        col = jax.lax.broadcasted_iota(jnp.int32, (H, 512), 1)
        sv = jnp.where(col < 512 - 48, sv, NEG)
      if q in (0, 2):
        held[q] = sv
        return
      hh = q // 2
      sa, sb = held[q - 1], sv
      mx = jnp.max(jnp.maximum(sa, sb), axis=-1, keepdims=True)
      mo = at.m[hh]
      mn = mx if mo is None else jnp.maximum(mo, mx)
      pa, pb = jnp.exp2(sa - mn), jnp.exp2(sb - mn)
      ta, tb = [(u[:, 0:128] + u[:, 128:256]) + (u[:, 256:384] + u[:, 384:512]) for u in (pa, pb)]
      if mo is None:
        at.al[hh] = None
        at.l[hh] = ta + tb
      else:
        at.al[hh] = jnp.exp2(mo - mn)
        at.l[hh] = at.l[hh] * at.al[hh] + (ta + tb)
      at.m[hh] = mn
      p[q - 1], p[q] = pa, pb
      for t_ in ((ta, tb) if hh == 0 else (tb, ta)):
        bd.push(row_vregs(t_), 12, hi=True)
      if c < 3:
        bd.push(row_vregs(at.l[hh]), 4, hi=True)
    return cb

  def att_carried(bd, at):
    p = [None] * 4
    cb = soft_cb(bd, at, 0, p)
    for q in range(4):
      cb(q, sS[q])
    return p

  def att_step(bd, at, b, c, p, get_u, bn_, cn, act=True, pv_budget=0):
    if at.acc is None:
      go = Gamma()
    else:
      acc = at.acc
      go = Gamma([(lambda q=q: acc[q] * al[q // 2]) for q in range(4)])
    al = list(at.al)
    pv = consumer_thunks(bd, go, alpha_forms(*p), lambda j: ld_bf(G[b, PVMAP[j], c * 256:(c + 1) * 256, :]),
                         budget=pv_budget)
    res = None
    if get_u is not None:
      pn = [None] * 4
      gs = Gamma(transposed=True, on_final=soft_cb(bd, at, cn, pn) if act else None)
      run(interleave(s_thunks(bd, gs, get_u, bn_, cn), pv))
      res = pn if act else gs.result()
    else:
      run(pv)
    at.acc = go.result()
    return res

  LS = TM // 8

  def conv_outputs(U, ls, dwk, u0, u1):
    start = (U % TPB) == 0
    win = {}

    def inp(u):
      if u not in win:
        win[u] = gb[ls, pl.ds(8 + u, 8, stride=LS), :]
      return win[u]

    outs = []
    for u in range(u0, u1):
      acc = [None, None]
      for k in range(KW):
        ui = u + k - KW // 2
        v = inp(ui)
        if start and u < 15 and ((u < 8) != (ui < 8)):
          v = jnp.where(sub0, 0.0, v)
        t = v * dwk[k]
        acc[k & 1] = t if acc[k & 1] is None else acc[k & 1] + t
      outs.append(acc[0] + acc[1])
    return outs

  def conv_unit(bd, U, lanes=(0, 1, 2, 3)):
    ru = (U + 1) * TM
    bounds = [(LS * g + NG // 2) // NG for g in range(NG + 1)]

    def make(l):
      ls = slice(l * 128, (l + 1) * 128)
      state = {}

      def group(g, anchor):
        u0, u1 = bounds[g], bounds[g + 1]
        dwk = [DWB[k, :, ls] for k in range(KW)]
        if anchor is not None:
          dwk = [bd.gate(v, anchor) for v in dwk]
        outs = conv_outputs(U, l, dwk, u0, u1)
        if g == 0:
          if U == 0:
            st[0:8, ls] = outs[8]
          state["k"] = outs[8] if U == 0 else st[0:8, ls]
          state["s1"] = st[8:16, ls]
          state["s2"] = st[16:24, ls]
        deps = []
        for u, o in zip(range(u0, u1), outs):
          d = o - state["k"]
          if U == 0 and u < 8:
            d = jnp.where(sub0, 0.0, d)
          d2 = d * d
          state["s1"] = state["s1"] + d
          state["s2"] = state["s2"] + d2
          dc[l, pl.ds(ru + u, 8, stride=LS), :] = o
          deps.append(d2)
        deps.append(dc[l, pl.ds(ru + u1 - 1, 8, stride=LS), :])
        if g == NG - 1:
          st[8:16, ls] = state["s1"]
          st[16:24, ls] = state["s2"]
        return deps
      return group

    for l in lanes:
      grp = make(l)
      for g in range(NG):
        n = bounds[g + 1] - bounds[g]
        bd.push_lazy(W_CONV * n + 15, n + 1, lambda a, grp=grp, g=g: grp(g, a))

  def conv_part(win, nr, dwk):
    acc = [None, None]
    for rho in range(8):
      if rho == 0:
        tt = win[8:8 + nr] * rep(dwk[7], nr // 8, 0)
      else:
        u = (win[0:nr + 8] * rep(dwk[rho - 1], nr // 8 + 1, 0)
             + win[8:nr + 16] * rep(dwk[rho + 7], nr // 8 + 1, 0))
        tt = pltpu.roll(u, nr + 8 - rho, 0)[0:nr]
      acc[rho & 1] = tt if acc[rho & 1] is None else acc[rho & 1] + tt
    return acc[0] + acc[1]

  def conv_exposed(bd, U, lanes):
    keep = bd.hi, bd.lo
    bd.hi, bd.lo = [], []
    conv_unit(bd, U, lanes)
    for _, _, fn in bd.lo:
      fn(None)
    bd.hi, bd.lo = keep

  def conv_tail(lanes):
    for l in lanes:
      ls = slice(l * 128, (l + 1) * 128)
      dwk = [DWB[k, :, ls] for k in range(KW)]
      halo = gb[l, TM:TM + 16, :]
      w = jnp.concatenate([halo, jnp.zeros((8, 128), F32)], axis=0)
      out = conv_part(w, 8, dwk)
      dc[l, N + TM:N + TM + 8, :] = out
      d = out - st[0:8, ls]
      st[8:16, ls] = st[8:16, ls] + d
      st[16:24, ls] = st[16:24, ls] + d * d

  def epi_mvo(bd, t, budget=0):
    r = mult(t * TM, TM)
    rl = [1.0 / jnp.sum(lsc[hh], axis=-1, keepdims=True) for hh in range(2)]
    oq = [osc[0] * rl[0], osc[1] * rl[0], osc[2] * rl[1], osc[3] * rl[1]]
    g = Gamma(init_quads(x1, r))
    run(consumer_thunks(bd, g, alpha_forms(*oq), lambda j: ld_bf(MVO[j]), budget=budget))
    y = g.result()
    xs = [jnp.concatenate([y[0], y[1]], axis=1), jnp.concatenate([y[2], y[3]], axis=1)]
    for h, v in zip((0, H), xs):
      store_tied(bd, x1, (), r + h, 0, v, 80)
    return [ln_rows(v) for v in xs]

  def epi_pw1(bd, ha, hb, sl, cache, budget=0, pre_store=None):
    g = Gamma()
    run(consumer_thunks(bd, g, alpha_forms(*quads(ha, hb)),
                        lambda j: ld_bf(WP1[j, :, sl * 256:(sl + 1) * 256]), order=AORD, cache=cache,
                        budget=budget))
    if pre_store is not None:
      pre_store()
    a1, b1, a2, b2 = g.result()
    deps = []
    for h, gv in ((0, a1 + a1 * jnp.tanh(b1)), (H, a2 + a2 * jnp.tanh(b2))):
      for k in range(2):
        gb[2 * sl + k, 16 + h:16 + h + H, :] = gv[:, k * 128:(k + 1) * 128]
        deps += [gb[2 * sl + k, r:r + 8, :] for r in range(16 + h, 16 + h + H, 8)]
    return deps

  def pre3(bd, t):
    r = mult(t * TM, TM)
    mu = rep(bn[0:8, :], H // 8, 0)
    hrs = rep(bn[8:16, :], H // 8, 0)
    hs = [half_silu((jnp.concatenate([dc[l, pl.ds(r + TM + 8 + h, H), :] for l in range(4)], axis=1)
                     - mu) * hrs) for h in (0, H)]
    for u in hs:
      bd.push(row_vregs(jnp.maximum(jnp.maximum(u[:, 0:128], u[:, 128:256]),
                                    jnp.maximum(u[:, 256:384], u[:, 384:512]))), 24, hi=True)
    g = Gamma(init_quads(x1, r))
    holder = []

    def finish():
      y = g.result()
      xs = [jnp.concatenate([y[0], y[1]], axis=1), jnp.concatenate([y[2], y[3]], axis=1)]
      ha, hb = [ln_rows(v) for v in xs]
      bd.lo[0:0] = [(W_LN, 1, (lambda a, d=d: [d])) for d in ln_deps(ha, hb)]
      for h, v in zip((0, H), xs):
        store_tied(bd, x1, (), r + h, 0, v, 80)
      holder.extend([ha, hb])

    return consumer_thunks(bd, g, alpha_forms(*quads(*hs)), lambda j: ld_bf(WP2[j])) + [finish], holder

  def post3(bd, t):
    r = mult(t * TM, TM)

    def piece(r0, anchor):
      x = x1[pl.ds(r + r0, LNR), :]
      if anchor is not None and LNGATE:
        x = bd.gate(x, anchor)
      o = ln_rows(x)
      xo[pl.ds(r + r0, LNR), :] = o.astype(BF)
      got = pltpu.bitcast(xo[pl.ds(r + r0 + LNR - 16, 16), 0:128], U32)
      return row_vregs(o, 384) + [pltpu.bitcast(got, F32)]

    for r0 in range(0, TM, LNR):
      bd.push_lazy((W_LN + 4) * (LNR // 8), LNR // 8 + 1, lambda a, r0=r0: piece(r0, a))

  sub0 = jax.lax.broadcasted_iota(jnp.int32, (8, 128), 0) == 0

  def zero_step(j, c):
    for b in range(NB):
      G[b, j, T // 4:1024, :] = jnp.zeros((1024 - T // 4, 256), U32)
    return c
  jax.lax.fori_loop(0, 7, zero_step, 0)

  def zero_rows(i, c):
    r = mult(i * 48, 8)
    gb[:, pl.ds(r, 48), :] = jnp.zeros((4, 48, 128), F32)
    x1[pl.ds(r, 48), :] = jnp.zeros((48, D), F32)
    return c
  jax.lax.fori_loop(0, (TM + 16) // 48, zero_rows, 0)
  st[...] = jnp.zeros(st.shape, F32)

  wcopy(I_Q).wait()
  wcopy(I_K).wait()
  prep_from_value(dot_nt(rq[...], rk[...]) * QSCALE, MQK)
  wcopy(I_V).wait()
  wcopy(I_O).wait()
  wcopy(I_B1).start()
  xcopy(1).start()
  prep_from_value(dot(rv[...], ro[...]), MVO)
  xcopy(0).wait()
  zs[...] = pltpu.bitcast(xo[0:16, 0:128], U32) >> 31
  wcopy(I_A1).wait()

  def prep_wa1(i, c):
    c0 = mult(i * 256, 256)
    blk = [ra1[r:r + 256, pl.ds(c0 + cc, 256)].astype(F32) * 0.5 for r in (0, 256) for cc in (0, 1024)]
    for j, f in enumerate(beta_forms(*blk)):
      WA[j, :, pl.ds(c0, 256)] = st_bf(f())
    return c
  jax.lax.fori_loop(0, 4, prep_wa1, 0)
  bd = Body()
  ha, hb = [ln_rows(v.astype(F32)) for v in rows2(xo, 0)]
  wcopy(I_B1).wait()
  for t in range(2, NT):
    xcopy(t).start()
  for i in (I_P1, I_DW, I_P2, I_A2, I_B2):
    wcopy(i).start()
  bd.push(prep_weight(rb1, WB, 1024, 256, 0.5), W_PREP)
  gz = Gamma()
  run(ff_a(bd, gz, fresh_u(alpha_forms(*quads(ha, hb))), 0))
  for k, v in enumerate(gz.result()):
    sS[k] = half_silu(v) if k < 3 else v

  def p1_body(t, last):
    bd = Body(BUD1, NHI1)
    r0 = mult(t * TM, TM)
    if not last:
      xcopy(t + 1).wait()
      rn = mult((t + 1) * TM, TM)
      lnx = LazyLN(bd, lambda h, r0: xo[pl.ds(rn + h * H + r0, LNR), :].astype(F32))
    post_g(bd, max(t - 1, 0) if isinstance(t, int) else jnp.maximum(t - 1, 0))
    gy = Gamma(init_quads(xo, r0, cast=True), reps=2)
    p = ff_step(bd, 0, ff_carried(bd), scratch_u, 1, gy, True)
    if not last:
      z = ff_step(bd, 1, p, fresh_u(alpha_forms(*quads(*lnx.get()))), 0, gy, False)
      store_quads(x1, r0, gy.result())
      for k in range(4):
        sS[k] = z[k]
    else:
      bth = ff_b(bd, gy, p, 1)
      gq = Gamma()
      run(merge(qp_thunks(bd, gq, 0), bth[:3]))
      gs = Gamma(transposed=True)
      run(merge(s_thunks(bd, gs, fresh_u(phi_forms(*gq.result())), 0, 0), bth[3:]))
      store_quads(x1, r0, gy.result())
      for k, v in enumerate(gs.result()):
        sS[k] = v
    bd.flush()

  jax.lax.fori_loop(0, NT - 1, lambda t, c: (p1_body(t, False), c)[1], 0)
  p1_body(NT - 1, True)

  def p2_body(i, first, last):
    bd = Body(BUD2, NHI2)
    b = i // TPB
    bn_ = (i + 1) // TPB
    at = Att()
    if first:
      for k in (I_P1, I_DW, I_P2, I_A2, I_B2):
        wcopy(k).wait()
      post_g(bd, NT - 1)
      dwf = rdw[...].astype(F32)
      for k in range(KW):
        DWB[k] = jnp.broadcast_to(dwf[k:k + 1, :], (8, D))
      bd.push(prep_weight(rp1, WP1, 256, 512, 0.5), W_PREP)
      bd.push(prep_weight(rp2, WP2, 256, 256, 1.0), W_PREP)
      bd.push(prep_weight(ra2, WA, 256, 1024, 0.5), W_PREP)
      bd.push(prep_weight(rb2, WB, 1024, 256, 0.5), W_PREP)
    else:
      conv_unit(bd, i - 2)
      halo = gb[:, TM:TM + 16, :]
    s = att_step(bd, at, b, 0, att_carried(bd, at), scratch_u, b, 1)
    if not first:
      ha, hb = epi_mvo(bd, i - 1, budget=BUDM)
    s = att_step(bd, at, b, 1, s, scratch_u, b, 2)
    if not first:
      bd.push(ln_deps(ha, hb), W_LN)
    s = att_step(bd, at, b, 2, s, scratch_u, b, 3)
    if not first:
      cache = {}

      def roll_window():
        bd.flush_lo()
        gb[:, 0:16, :] = halo

      gd = epi_pw1(bd, ha, hb, 0, cache, budget=BUDP, pre_store=roll_window)
      gd += epi_pw1(bd, ha, hb, 1, cache)
      if not last:
        bd.push(gd, 8)
    if not last:
      gq = Gamma()
      run(qp_thunks(bd, gq, i + 1))
      s = att_step(bd, at, b, 3, s, fresh_u(phi_forms(*gq.result())), bn_, 0, False)
      for k in range(4):
        sS[k] = s[k]
    else:
      conv_unit(bd, i - 1, HOST8)
      att_step(bd, at, b, 3, s, None, None, None, pv_budget=BUDL)
    for k in range(4):
      osc[k] = at.acc[k]
    for hh in range(2):
      lsc[hh] = at.l[hh]
    if first:
      bd.flush()
    return bd

  p2_body(0, True, False)
  def p2_pair(k, c):
    p2_body(2 * k + 1, False, False)

    @pl.when(k >= 0)
    def _():
      p2_body(2 * k + 2, False, False)
    return c
  for i_ in range(1, NT - 1):
    p2_body(i_, False, False)
  bd = p2_body(NT - 1, False, True)

  ha, hb = epi_mvo(bd, NT - 1, budget=BUDL2)

  def roll_window():
    bd.flush()
    conv_exposed(bd, NT - 2, [l for l in range(4) if l not in HOST8])
    gb[:, 0:16, :] = gb[:, TM:TM + 16, :]

  epi_pw1(bd, ha, hb, 0, None, budget=BUDL2, pre_store=roll_window)
  conv_unit(bd, NT - 1, HOSTL)
  epi_pw1(bd, ha, hb, 1, None, budget=BUDL3)
  bd.flush()
  conv_exposed(bd, NT - 1, [l for l in range(4) if l not in HOSTL])
  conv_tail((0, 1, 2, 3))
  n_s = jnp.where(jax.lax.broadcasted_iota(jnp.int32, (8, D), 0) == 0, N // 8 - 7.0, N // 8 + 1.0)
  s1 = st[8:16, :]
  mu_s = st[0:8, :] + s1 / n_s
  m2_s = st[16:24, :] - s1 * s1 / n_s
  mu = jnp.sum(mu_s * n_s, axis=0, keepdims=True) * (1.0 / N)
  dm = mu_s - mu
  var = jnp.sum(m2_s + dm * dm * n_s, axis=0, keepdims=True) * (1.0 / N)
  bn[0:8, :] = jnp.broadcast_to(mu, (8, D))
  bn[8:16, :] = jnp.broadcast_to(0.5 * jax.lax.rsqrt(var + EPS), (8, D))

  bd = Body()
  th, (hold) = pre3(bd, 0)
  run(th)
  ha, hb = hold
  gz = Gamma()
  run(ff_a(bd, gz, fresh_u(alpha_forms(*quads(ha, hb))), 0))
  for k, v in enumerate(gz.result()):
    sS[k] = half_silu(v) if k < 3 else v

  def p3_body(t, last):
    bd = Body(BUD3, NHI3)
    r0 = mult(t * TM, TM)

    @pl.when(t >= 2)
    def _():
      ocopy(t - 2).start()

    p0 = ff_carried(bd)
    extra = None
    if not last:
      th, hold = pre3(bd, t + 1)
      extra = (P3POS, th)
    post3(bd, max(t - 1, 0) if isinstance(t, int) else jnp.maximum(t - 1, 0))
    gy = Gamma(init_quads(x1, r0), reps=2)
    p = ff_step(bd, 0, p0, scratch_u, 1, gy, True, extra)
    if not last:
      z = ff_step(bd, 1, p, fresh_u(alpha_forms(*quads(*hold))), 0, gy, False)
      for k in range(4):
        sS[k] = z[k]
    else:
      run(ff_b(bd, gy, p, 1))
    store_quads(x1, r0, gy.result())
    bd.flush()

  jax.lax.fori_loop(0, NT - 1, lambda t, c: (p3_body(t, False), c)[1], 0)
  p3_body(NT - 1, True)

  bd = Body()
  ocopy(NT - 2).start()
  post3(bd, NT - 1)
  bd.flush()
  ocopy(NT - 1).start()
  for t in range(NT):
    ocopy(t).wait()


@jax.jit
def pallas_standalone__conformer_family_conformer__speech_kernel(
    x, w_ff1_a, w_ff1_b, w_q, w_k, w_v, w_o, w_pw1, dw, w_pw2, w_ff2_a, w_ff2_b):
  hbm = pl.BlockSpec(memory_space=pl.ANY)
  V = pltpu.VMEM
  out = pl.pallas_call(
      kernel,
      out_shape=jax.ShapeDtypeStruct((N, D), x.dtype),
      in_specs=[hbm] * 12,
      out_specs=hbm,
      scratch_shapes=[
          V((N, D), BF),
          V((D, FH), BF), V((FH, D), BF), V((D, FH), BF), V((FH, D), BF),
          V((D, D), BF), V((D, D), BF), V((D, D), BF), V((D, D), BF),
          V((D, 2 * D), BF), V((KW, D), BF), V((D, D), BF),
          V((7, 128, 1024), U32), V((7, 512, 256), U32),
          V((7, 128, 256), U32), V((7, 128, 256), U32),
          V((7, 128, 512), U32), V((7, 128, 256), U32),
          V((KW, 8, D), F32),
          V((N, D), F32),
          V((4, N + TM + 8, 128), F32),
          V((NB, 7, 1024, 256), U32),
          V((4, TM + 16, 128), F32),
          V((4, H, 512), F32),
          V((7, H // 2, 256), U32),
          V((4, H, 256), F32),
          V((2, H, 128), F32),
          V((24, D), F32), V((16, D), F32), V((8, 128), U32),
          pltpu.SemaphoreType.DMA((2 * NT + 11,)),
      ],
      compiler_params=pltpu.CompilerParams(vmem_limit_bytes=124 * 1024 * 1024),
  )(x.reshape(N, D), w_ff1_a, w_ff1_b, w_q, w_k, w_v, w_o, w_pw1, dw, w_pw2, w_ff2_a, w_ff2_b)
  return out.reshape(NB, T, D)
```
